```python
import os as _os
_os.environ.setdefault("JAX_PLATFORMS", "cpu")
import jax
import jax.numpy as jnp

def _softmax(x, axis=-1):
    return jax.nn.softmax(x, axis=axis)
def _gelu(x):
    return jax.nn.gelu(x, approximate=True)
def _silu(x):
    return jax.nn.silu(x)
def _sigmoid(x):
    return jax.nn.sigmoid(x)
def _layernorm(x, axis=-1, eps=1e-5):
    m = jnp.mean(x, axis=axis, keepdims=True)
    v = jnp.var(x, axis=axis, keepdims=True)
    return (x - m) / jnp.sqrt(v + eps)
def _scatter_add(tgt, idx, src, axis=0):
    return tgt.at[idx].add(src)
def _segment_sum(src, seg, n):
    return jax.ops.segment_sum(src, seg, n)
class _Rng:
    def __init__(self, key):
        self._k = key
    def _next(self):
        self._k, sub = jax.random.split(self._k)
        return sub
    def normal(self, shape):
        return jax.random.normal(self._next(), shape, dtype=jnp.bfloat16)
    def randint(self, lo, hi, shape):
        return jax.random.randint(self._next(), shape, lo, hi, dtype=jnp.int32)
    def uniform(self, shape, lo=0.0, hi=1.0):
        return jax.random.uniform(self._next(), shape, jnp.bfloat16, lo, hi)
    def permutation(self, n):
        return jax.random.permutation(self._next(), n)


kernel_name = 'interleave_layers__linear_attn_block__mha_block__prompt'

def setup_inputs():
    _rng = _Rng(jax.random.key(int.from_bytes(__import__("os").urandom(4), "little")))
    _w = (lambda a: (lambda t: t.astype(jnp.bfloat16) if jnp.issubdtype(t.dtype, jnp.floating) else t)(jnp.asarray(a)))
    def _A_setup():
        B, S, D = 1, 2048, 1024
        return {
            "x": _w((lambda *s: _rng.normal(s) * 0.05)(B, S, D)),
            "wqkv": _w((lambda *s: _rng.normal(s) * 0.1)(D, 3 * D)),
            "wo": _w((lambda *s: _rng.normal(s) * 0.1)(D, D)),
        }
    _A_in = _A_setup()

    def _B_setup():
        B, S, D, H = 1, 2048, 1024, 32
        return {
            "x": _w((lambda *s: _rng.normal(s) * 0.05)(B, S, D)),
            "wqkv": _w((lambda *s: _rng.normal(s) * 0.1)(D, 3 * D)),
            "wo": _w((lambda *s: _rng.normal(s) * 0.05)(D, D)),
        }
    _B_in = _B_setup()

    return {
        "A_x": _A_in["x"],
        "A_wqkv": _A_in["wqkv"],
        "A_wo": _A_in["wo"],
        "B_x": _B_in["x"],
        "B_wqkv": _B_in["wqkv"],
        "B_wo": _B_in["wo"],
    }

def reference(A_x, A_wqkv, A_wo, B_x, B_wqkv, B_wo):
    def _A_ref(x, wqkv, wo):
        B, S, D = x.shape
        H = 32; Dh = D // H
        qkv = (lambda x, *d: x.transpose(*d))((x @ wqkv).reshape(B, S, 3, H, Dh), 2, 0, 3, 1, 4)
        q, k, v = qkv[0], qkv[1], qkv[2]
        phi = lambda t: jnp.where(t > 0, t + 1, jnp.exp(t)) + 1e-6
        pq, pk = phi(q), phi(k)
        kv = jnp.einsum("bhsd,bhse->bhde", pk, v)
        z = jnp.einsum("bhsd->bhd", pk)
        num = jnp.einsum("bhqd,bhde->bhqe", pq, kv)
        den = jnp.einsum("bhqd,bhd->bhq", pq, z)[..., None] + 1e-6
        o = num / den
        return (lambda x, *d: x.transpose(*d))(o, 0, 2, 1, 3).reshape(B, S, D) @ wo

    def _B_ref(x, wqkv, wo):
        B, S, D = x.shape
        H = 32
        Dh = D // H
        qkv = (lambda x, *d: x.transpose(*d))((x @ wqkv).reshape(B, S, 3, H, Dh), 2, 0, 3, 1, 4)
        q, k, v = qkv[0], qkv[1], qkv[2]
        scores = jnp.einsum("bhqd,bhkd->bhqk", q, k) * (Dh ** -0.5)
        p = _softmax(scores, axis=-1)
        o = jnp.einsum("bhqk,bhkd->bhqd", p, v)
        return (lambda x, *d: x.transpose(*d))(o, 0, 2, 1, 3).reshape(B, S, D) @ wo

    x = A_x
    x = x + _A_ref(_layernorm(x, axis=-1), A_wqkv, A_wo)
    x = x + _B_ref(_layernorm(x, axis=-1), B_wqkv, B_wo)
    x = x + _A_ref(_layernorm(x, axis=-1), A_wqkv, A_wo)
    x = x + _B_ref(_layernorm(x, axis=-1), B_wqkv, B_wo)
    return x
```

```python
import math

import jax
import jax.numpy as jnp
from jax import lax
from jax.experimental import pallas as pl
from jax.experimental.pallas import tpu as pltpu

f32, bf16, u32 = jnp.float32, jnp.bfloat16, jnp.uint32

S, D, H, DH = 2048, 1024, 32, 32
NG = D // 128
QB = 512
KB = 128
NS = S // KB
RB = 512
NRB = S // RB
MQ, KQ = RB // 4, D // 4
NPROD = 49
ATT_U = 1
ONLY = None
TPP = 4
FLAG = 4
AHEAD = 2
FS1 = 0.45
FS2 = 0.55
LN_GAP = 3
LN_ROWS = 8
QSCALE = math.log2(math.e) * DH ** -0.5
W_AQ, W_AK, W_AV, W_AO, W_BQ, W_BK, W_BV, W_BO = range(8)

LHS_TERMS = [[(1, 0, 0), (1, 1, 1)], [(1, 1, 0), (1, 1, 1)], [(1, 0, 0)], [(1, 1, 1)],
             [(1, 0, 0), (1, 0, 1)], [(1, 1, 0), (-1, 0, 0)], [(1, 0, 1), (-1, 1, 1)]]
RHS_TERMS = [[(1, 0, 0), (1, 1, 1)], [(1, 0, 0)], [(1, 0, 1), (-1, 1, 1)], [(1, 1, 0), (-1, 0, 0)],
             [(1, 1, 1)], [(1, 0, 0), (1, 0, 1)], [(1, 1, 0), (1, 1, 1)]]
ORDER = (0, 1, 3, 4, 2, 6, 5)


def _tree(xs, op):
    xs = list(xs)
    while len(xs) > 1:
        xs = [op(xs[i], xs[i + 1]) if i + 1 < len(xs) else xs[i] for i in range(0, len(xs), 2)]
    return xs[0]


def _fold8(acc, x, op):
    x = _tree([x[8 * i:8 * i + 8] for i in range(x.shape[0] // 8)], op)
    return x if acc is None else op(acc, x)


def _dot(a, b):
    return jnp.dot(a, b, preferred_element_type=f32)


def _phi(t):
    return jnp.where(t > 0, t + 1.0, jnp.exp(t)) + 1e-6


def _form(terms, block):
    x = block(terms[0][1], terms[0][2])
    for s, r, c in terms[1:]:
        x = x + block(r, c) if s > 0 else x - block(r, c)
    return x


def _forms(table, i, block):
    q = {(r, c): _form(table[i], lambda ro, co: block(2 * ro + r, 2 * co + c)) for r in range(2) for c in range(2)}
    return [_form(t, lambda r, c: q[r, c]) for t in table]


def _strassen(prod, sink, lev=2, base=0):
    if lev == 0:
        return prod(base, lambda g, m: sink(0, 0, g, m))
    h = 2 ** (lev - 1)
    m1, m2, m5, c11, c22 = {}, {}, {}, {}, {}
    run = lambda i, fn: _strassen(prod, fn, lev - 1, base + i * 7 ** (lev - 1))

    def got4(r, c, g, m):
        sink(h + r, c, g, m2[r, c, g] + m)
        c11[r, c, g] = m1[r, c, g] + m

    def got3(r, c, g, m):
        sink(r, h + c, g, m5[r, c, g] + m)
        c22[r, c, g] = m + m1[r, c, g] - m2[r, c, g]

    run(0, lambda r, c, g, m: m1.update({(r, c, g): m}))
    run(1, lambda r, c, g, m: m2.update({(r, c, g): m}))
    run(3, got4)
    run(4, lambda r, c, g, m: m5.update({(r, c, g): m}))
    run(2, got3)
    run(6, lambda r, c, g, m: sink(r, c, g, m + c11[r, c, g] - m5[r, c, g]))
    run(5, lambda r, c, g, m: sink(h + r, h + c, g, m + c22[r, c, g]))


def _tiles(sink, pre=lambda c, y: y):
    parts = {}

    def part(r, c, g, y):
        parts.setdefault((r, c), []).append(pre(c, y))
        if g == TPP - 1:
            y = jnp.concatenate(parts.pop((r, c)), axis=0)
            for t in range(2):
                sink(2 * c + t, r, y[:, 128 * t:128 * t + 128])
    return part


class _Side:
    def __init__(self, jobs, span, start=0):
        self.jobs, self.span, self.n, self.done = list(jobs), span, -start, 0

    def tick(self, fence):
        self.n += 1
        while self.done < len(self.jobs) and (self.done + 1) * self.span <= self.n * len(self.jobs):
            self.jobs[self.done](fence)
            self.done += 1


def _staggered(gens, phases):
    def job(n):
        for k in reversed(range(phases)):
            if 0 <= n - k < len(gens):
                next(gens[n - k], None)
    return [lambda n=n: job(n) for n in range(len(gens) + phases - 1)]


def _run(jobs):
    for job in jobs:
        job(lambda ref: None)


def _kernel(x_hbm, wa_hbm, woa_hbm, wb_hbm, wob_hbm, out_hbm,
            wf, af, woa, raw, xio, xr, st, oc, pv, kv, zs, zb, qT, kk, vT, sb, pc, sem):
    lane_head = lax.broadcasted_iota(jnp.int32, (128, 128), 1) // DH
    row_head = lax.broadcasted_iota(jnp.int32, (128, 128), 0) // DH
    same_head = lane_head == row_head
    on = lambda name: ONLY is None or name in ONLY
    RG = MQ // TPP
    T7 = 7 * TPP
    x_fence, st_fence, oc_fence = xr.at[S:S + 8, 0:128], st.at[RB:RB + 8, 0:128], oc.at[32, 0:8, 0:128]

    def packed(ref, *idx):
        return pltpu.bitcast(ref.bitcast(u32)[idx], bf16)

    pending = []

    def project(w, sides, sink):
        def prod(p, done):
            y = _dot(jnp.concatenate([packed(af, p, c) for c in range(2)], axis=1),
                     jnp.concatenate([packed(wf, w, p, c) for c in range(2)], axis=1))
            for g in range(TPP):
                fence = lambda ref: None
                if len(pending) >= FLAG:
                    fn, g0, y0 = pending.pop(0)
                    fn(g0, y0)

                    def fence(ref, y0=y0):
                        ref[...] = y0[0:ref.shape[0], 0:128].astype(ref.dtype)
                for side in sides:
                    side.tick(fence)
                pending.append((done, g, y[g * RG:(g + 1) * RG]))
        _strassen(prod, sink)

    def drain():
        while pending:
            fn, g, y = pending.pop(0)
            fn(g, y)

    def fenced(ref, jobs):
        def run(fence, job):
            fence(ref)
            job()
        return [lambda fence, job=job: run(fence, job) for job in jobs]

    def at(r, c, g):
        return slice(r * MQ + g * RG, r * MQ + (g + 1) * RG), slice(c * KQ, (c + 1) * KQ)

    def blk(i):
        return pl.ds(pl.multiple_of(i * RB, RB), RB)

    def lhs_jobs(b, groups):
        src = st.at[blk(b)]

        def job(p, c, i):
            tile = lambda r, k: src[r * MQ + 16 * p:r * MQ + 16 * p + 16, k * KQ + 128 * c:k * KQ + 128 * c + 128]
            for j, f in enumerate(_forms(LHS_TERMS, i, tile)):
                af[7 * i + j, c, 16 * p:16 * p + 16, :] = f.astype(bf16)

        return fenced(st_fence, [lambda p=p, c=c, i=i: job(p, c, i)
                                 for i in groups for p in range(MQ // 16) for c in range(2)])

    def operand_sides(zero, fill, nmat, share):
        span = 7 * nmat * T7
        per = int(T7 * min(1.0, nmat * (1.0 - share)))
        a, b = (7 - AHEAD) * per, span - AHEAD * per
        return [_Side(lhs_jobs(zero, ORDER[AHEAD:]), a), _Side(fill, b - a - 4, a), _Side(lhs_jobs(zero, ORDER[:AHEAD]), span - b - 2, b)]

    def rhs_jobs(w, tile16, r):
        def job(c, i):
            for j, f in enumerate(_forms(RHS_TERMS, i, lambda a, b: tile16(a * KQ + r, b * KQ + 128 * c))):
                wf[w, 7 * i + j, c, pl.ds(r, 16), :] = f.astype(bf16)
        return [lambda c=c, i=i: job(c, i) for c in range(2) for i in range(7)]

    def raw_tile(t):
        return lambda r, k: raw[pl.ds(pl.multiple_of(t * D + r, 16), 16), k:k + 128].astype(f32)

    def norm_jobs(i):
        x = xr.at[blk(i)]

        def rows(r):
            mu = jnp.mean(x[r, :], axis=-1, keepdims=True)
            for _ in range(LN_GAP):
                yield
            xc = x[r, :] - mu
            rstd = lax.rsqrt(jnp.mean(xc * xc, axis=-1, keepdims=True) + 1e-5)
            for _ in range(LN_GAP):
                yield
            st[r, :] = (x[r, :] - mu) * rstd
        return fenced(x_fence, _staggered([rows(slice(r, r + LN_ROWS)) for r in range(0, RB, LN_ROWS)], 2 * LN_GAP + 1))

    def front_jobs(denominator, i):
        def job(g, r):
            it, cols = g * 4 + i, slice(r, r + 128)
            o = []
            for h in range(4):
                x = oc[it, DH * h:DH * h + DH, cols]
                o.append(x * (1.0 / denominator(x, g, it, h, cols)))
            st[r:r + 128, 128 * g:128 * g + 128] = jnp.concatenate(o, axis=0).T
        return fenced(oc_fence, [lambda g=g, r=r: job(g, r) for g in range(NG) for r in range(0, RB, 128)])

    def lin_den(x, g, it, h, cols):
        return jnp.sum(_fold8(None, x * zb[g, DH * h:DH * h + DH, :], jnp.add), axis=0, keepdims=True) + 1e-6

    def att_den(x, g, it, h, cols):
        return jnp.sum(oc[it, 128 + 8 * h:136 + 8 * h, cols], axis=0, keepdims=True)

    def out_copy(i):
        return pltpu.make_async_copy(xio.at[blk(i)], out_hbm.at[blk(i)], sem.at[i])

    def out_project(w, den, zero, emit):
        def block(i, fill, share):
            def sink(r, c, g, y):
                y = xr.at[blk(i)][at(r, c, g)] + y
                xr.at[blk(i)][at(r, c, g)] = y
                if emit:
                    xio.at[blk(i)][at(r, c, g)] = y.astype(bf16)

            project(w, operand_sides(zero, fill, 1, share), sink)
            drain()
            if emit:
                out_copy(i).start()

        _run(front_jobs(den, 0) + lhs_jobs(zero, ORDER[:AHEAD]))
        lax.fori_loop(0, NRB - 1, lambda i, c: block(i, front_jobs(den, i + 1), FS1), None)
        block(zero + NRB - 1, norm_jobs(zero), FS2)

    def x_copy(i):
        return pltpu.make_async_copy(x_hbm.at[blk(i)], xio.at[blk(i)], sem.at[i])

    def w_copy(src, c, t):
        return pltpu.make_async_copy(src.at[:, pl.ds(c * D, D)], raw.at[pl.ds(t * D, D)], sem.at[NRB + t])

    wa_cp = [w_copy(wa_hbm, 1, 0), w_copy(wa_hbm, 2, 1), w_copy(wa_hbm, 0, 2)]
    wb_cp = [w_copy(wb_hbm, 0, 0), w_copy(wb_hbm, 1, 1), w_copy(wb_hbm, 2, 2), w_copy(wob_hbm, 0, 3)]
    wo_cp = pltpu.make_async_copy(woa_hbm, woa, sem.at[NRB + 4])

    def widen(i):
        def body(j, c):
            r = pl.ds(pl.multiple_of(i * RB + j * 64, 64), 64)
            xr[r, :] = xio[r, :].astype(f32)
        x_copy(i).wait()
        lax.fori_loop(0, RB // 64, body, None)

    def prep(t, w):
        def body(j, c):
            for job in rhs_jobs(w, raw_tile(t), pl.multiple_of(j * 16, 16)):
                job()
        lax.fori_loop(0, KQ // 16, body, None)

    x_copy(0).start()
    wa_cp[0].start()
    widen(0)
    wa_cp[1].start()
    _run(norm_jobs(0) + lhs_jobs(0, ORDER[:AHEAD]))
    for t, w in enumerate([W_AK, W_AV, W_AQ]):
        wa_cp[t].wait()
        if t == 0:
            wa_cp[2].start()
        else:
            x_copy(t).start()
        prep(t, w)
    x_copy(3).start()
    for c in wb_cp + [wo_cp]:
        c.start()

    def layer(l, c):
        zero = l // 2
        kv[...] = jnp.zeros_like(kv)
        zs[...] = jnp.zeros_like(zs)

        def qkv_a(i, c):
            @pl.when(jnp.logical_and(l == 0, i < NRB - 1))
            def _():
                widen(i + 1)

            def phi_k(c, y):
                y = _phi(y)
                zs[:, c * KQ:(c + 1) * KQ] += _fold8(None, y, jnp.add)
                return y

            def got_k(g, r, y):
                pv[0, g, r] = y.T.astype(bf16)

            def got_v(r, c, g, y):
                for t in range(2):
                    pv[1, 2 * c + t, r, g * RG:(g + 1) * RG, :] = y[:, 128 * t:128 * t + 128].astype(bf16)

            def got_q(g, r, y):
                oc[g * 4 + i, 0:128, r * MQ:(r + 1) * MQ] = _phi(y.T)

            def summarise(g):
                kv[g] += _dot(jnp.concatenate([packed(pv, 0, g, r) for r in range(4)], axis=1),
                              pltpu.bitcast(pv.bitcast(u32)[1, g].reshape(RB // 2, 128), bf16))

            sides = operand_sides(zero, norm_jobs(jnp.minimum(i + 1, NRB - 1)), 3, 0.5)
            project(W_AK, sides, _tiles(got_k, phi_k))
            project(W_AQ, sides, _tiles(got_q))
            project(W_AV, sides, got_v)
            for g in range(NG):
                if g == NG // 2:
                    drain()
                summarise(g)

        with jax.named_scope("p0"):
            if on("p0"): lax.fori_loop(0, NRB, qkv_a, None)

        @pl.when(l == 0)
        def _():
            for c in wb_cp + [wo_cp]:
                c.wait()
            with jax.named_scope("prepb"):
                for t, w in enumerate([W_BQ, W_BK, W_BV, W_BO]):
                    prep(t, w)

        @pl.when(l == 1)
        def _():
            for i in range(NRB):
                out_copy(i).wait()

        with jax.named_scope("p1"):
          if on("p1"):
            z = jnp.sum(zs[...], axis=0, keepdims=True)
            wp = []
            for g in range(NG):
                cs = slice(128 * g, 128 * g + 128)
                zb[g] = jnp.broadcast_to(z[:, cs], (128, 128)).T
                wp.append(_dot(jnp.where(same_head, kv[g], 0.0).astype(bf16), woa[cs, :]))
            wp = jnp.concatenate(wp, axis=0)
            for j in range(KQ // 16):
                for job in rhs_jobs(W_AO, lambda r, k: wp[r:r + 16, k:k + 128], 16 * j):
                    job()
        with jax.named_scope("p2a"):
            if on("p2a"): out_project(W_AO, lin_den, zero, False)

        def qkv_b(i, c):
            def got_q(g, r, y):
                qT[g * 4 + i, :, r * MQ:(r + 1) * MQ] = y.T.astype(bf16)

            def got_v(g, r, y):
                vT[g, i * 4 + r] = y.T.astype(bf16)

            def got_k(r, c, g, y):
                for t in range(2):
                    kk[2 * c + t, i * 4 + r, g * RG:(g + 1) * RG, :] = y[:, 128 * t:128 * t + 128].astype(bf16)

            sides = operand_sides(zero, norm_jobs(jnp.minimum(i + 1, NRB - 1)), 3, 0.5)
            project(W_BQ, sides, _tiles(got_q, lambda c, y: y * QSCALE))
            project(W_BV, sides, _tiles(got_v))
            project(W_BK, sides, got_k)
            drain()

        with jax.named_scope("p2b"):
            if on("p2b"): lax.fori_loop(0, NRB, qkv_b, None)

        zq = jnp.zeros((DH, QB), bf16)

        def qk(it, h, j):
            q = qT[it, DH * h:DH * h + DH, :]
            q = jnp.concatenate([q if a == h else zq for a in range(4)], axis=0)
            return _dot(kk[it // 4, j], q)

        def fin_max(m):
            return jnp.broadcast_to(jnp.max(m, axis=0, keepdims=True), (8, QB))

        def expo(x, m):
            return jnp.exp2(x.reshape(x.shape[0] // 8, 8, QB) - m[None]).reshape(x.shape[0], QB)

        G = 32
        with jax.named_scope("p3"):
          if on("p3"):
            mn = None
            for n in range(NS + 1):
                h, j = divmod(n, NS)
                s = qk(0, h, j)
                sb[h, j * KB:(j + 1) * KB, :] = s
                if n == NS:
                    m, mn = fin_max(mn), None
                mn = _fold8(mn, s, jnp.maximum)
            p = expo(sb[0, 0:KB, :], m)
            pc[...] = p.astype(bf16)

            def p3(i, carry):
                m, mn, lsum = carry
                bufs = [sb.at[zero], sb.at[1 - zero]]
                p = pc[...]
                acc0 = jnp.full((DH, QB), zero.astype(f32))
                for u in range(ATT_U):
                    it = i * ATT_U + u
                    nit = jnp.minimum(it + 1, 31)
                    for n in range(4 * NS):
                        h, j = divmod(n, NS)
                        t1, j1 = divmod(n + NS + 1, NS)
                        t2, j2 = divmod(n + 1, NS)
                        s = qk(it if t1 < 4 else nit, t1 % 4, j1)
                        o = _dot(vT[it // 4, j, DH * h:DH * h + DH, :], p)
                        if j1 == 0:
                            m, mn = fin_max(mn), None
                            ldone, lsum = lsum, None
                        pp = [None] * (KB // G)
                        for g in range(KB // G):
                            sg = s[g * G:(g + 1) * G]
                            bufs[t1 % 2][j1 * KB + g * G:j1 * KB + g * G + G, :] = sg
                            mn = _fold8(mn, sg, jnp.maximum)
                            gg = KB // G - 1 - g
                            pp[gg] = expo(bufs[t2 % 2][j2 * KB + gg * G:j2 * KB + gg * G + G, :], m)
                            lsum = _fold8(lsum, pp[gg], jnp.add)
                        p = jnp.concatenate(pp, axis=0).astype(bf16)
                        acc = (acc0 if j == 0 else acc) + o
                        if j == NS - 1:
                            oc[it, DH * h:DH * h + DH, :] = acc
                            oc[it, 128 + 8 * h:136 + 8 * h, :] = ldone
                pc[...] = p
                return m, mn, lsum

            lax.fori_loop(0, 32 // ATT_U, p3, (m, mn, _fold8(None, p, jnp.add)))

        with jax.named_scope("p4a"):
            if on("p4a"): out_project(W_BO, att_den, zero, True)

    lax.fori_loop(0, 2, layer, None)
    for i in range(NRB):
        out_copy(i).wait()


@jax.jit
def pallas_interleave_layers__linear_attn_block__mha_block__prompt_kernel(
    A_x, A_wqkv, A_wo, B_x, B_wqkv, B_wo,
):
    del B_x
    assert A_x.shape == (1, S, D)
    out = pl.pallas_call(
        _kernel,
        name="fused",
        out_shape=jax.ShapeDtypeStruct((S, D), bf16),
        in_specs=[pl.BlockSpec(memory_space=pl.ANY)] * 5,
        out_specs=pl.BlockSpec(memory_space=pl.ANY),
        scratch_shapes=[
            pltpu.VMEM((8, NPROD, 2, KQ, 128), bf16),
            pltpu.VMEM((NPROD, 2, MQ, 128), bf16),
            pltpu.VMEM((D, D), bf16),
            pltpu.VMEM((4 * D + 16, D), bf16),
            pltpu.VMEM((S, D), bf16),
            pltpu.VMEM((S + 8, D), f32),
            pltpu.VMEM((RB + 8, D), f32),
            pltpu.VMEM((33, 160, QB), f32),
            pltpu.VMEM((2, NG, 4, 128, 128), bf16),
            pltpu.VMEM((NG, 128, 128), f32),
            pltpu.VMEM((8, D), f32),
            pltpu.VMEM((NG, 128, 128), f32),
            pltpu.VMEM((32, 128, QB), bf16),
            pltpu.VMEM((NG, NS, KB, 128), bf16),
            pltpu.VMEM((NG, NS, 128, KB), bf16),
            pltpu.VMEM((2, S, QB), f32),
            pltpu.VMEM((KB, QB), bf16),
            pltpu.SemaphoreType.DMA((NRB + 5,)),
        ],
        compiler_params=pltpu.CompilerParams(vmem_limit_bytes=124 * 2**20),
    )(A_x.reshape(S, D), A_wqkv, A_wo, B_wqkv, B_wo)
    return out.reshape(1, S, D)
```

```python
import math

import jax
import jax.numpy as jnp
from jax import lax
from jax.experimental import pallas as pl
from jax.experimental.pallas import tpu as pltpu

f32, bf16, u32 = jnp.float32, jnp.bfloat16, jnp.uint32

S, D, H, DH = 2048, 1024, 32, 32
NG = D // 128
QB = 512
KB = 128
NS = S // KB
RB = 512
NRB = S // RB
MQ, KQ = RB // 4, D // 4
NPROD = 49
ATT_U = 2
ONLY = None
TPP = 4
FLAG = 4
AHEAD = 2
HALF = 0
WK_SPLIT = ((0, 128), (128, 80), (208, 48))
TC = 122
TD = 64
RO = 2
RA = (0, 0, 3)
RBB = (0, 0, 3)
R2 = 10
LAYERS = (0, 1)
FS1 = 0.45
FS2 = 0.55
LN_GAP = 4
LN_ROWS = 8
QSCALE = math.log2(math.e) * DH ** -0.5
W_AQ, W_AK, W_AV, W_AO, W_BQ, W_BK, W_BV, W_BO = range(8)

LHS_TERMS = [[(1, 0, 0), (1, 1, 1)], [(1, 1, 0), (1, 1, 1)], [(1, 0, 0)], [(1, 1, 1)],
             [(1, 0, 0), (1, 0, 1)], [(1, 1, 0), (-1, 0, 0)], [(1, 0, 1), (-1, 1, 1)]]
RHS_TERMS = [[(1, 0, 0), (1, 1, 1)], [(1, 0, 0)], [(1, 0, 1), (-1, 1, 1)], [(1, 1, 0), (-1, 0, 0)],
             [(1, 1, 1)], [(1, 0, 0), (1, 0, 1)], [(1, 1, 0), (1, 1, 1)]]
ORDER = (0, 1, 3, 4, 2, 6, 5)


def _tree(xs, op):
    xs = list(xs)
    while len(xs) > 1:
        xs = [op(xs[i], xs[i + 1]) if i + 1 < len(xs) else xs[i] for i in range(0, len(xs), 2)]
    return xs[0]


def _fold8(acc, x, op):
    x = _tree([x[8 * i:8 * i + 8] for i in range(x.shape[0] // 8)], op)
    return x if acc is None else op(acc, x)


def _dot(a, b):
    return jnp.dot(a, b, preferred_element_type=f32)


def _phi(t):
    return jnp.where(t > 0, t + 1.0, jnp.exp(t)) + 1e-6


def _flip(table, rows, cols):
    return [[(s * (-1 if rows and r else 1) * (-1 if cols and c else 1), r, c) for s, r, c in t] for t in table]


def _signed_sum(terms):
    s0, x = terms[0]
    for s, v in terms[1:]:
        x = x + v if s == s0 else x - v
    return s0, x


def _forms(table, i, block):
    q = {(r, c): _signed_sum([(s, block(2 * ro + r, 2 * co + c)) for s, ro, co in table[i]])[1]
         for r in range(2) for c in range(2)}
    return [_signed_sum([(s, q[r, c]) for s, r, c in t])[1] for t in table]


def _strassen(kind, prod, sink, lev=2, base=0):
    if lev == 0:
        return prod(base, lambda g, m: sink(0, 0, g, m))
    h = 2 ** (lev - 1)
    lhs, rhs, low = kind
    sg = [a[0][0] * b[0][0] for a, b in zip(lhs, rhs)]
    m1, m2, m5, c11, c22 = {}, {}, {}, {}, {}
    run = lambda i, fn: _strassen(kind, prod, fn, lev - 1, base + i * 7 ** (lev - 1))

    def total(*terms):
        s, x = _signed_sum(sorted(terms, key=lambda t: -t[0]))
        assert s > 0
        return x

    def got4(r, c, g, m):
        sink(h + r, c, g, total((low * sg[1], m2[r, c, g]), (low * sg[3], m)))
        c11[r, c, g] = total((sg[0], m1[r, c, g]), (sg[3], m))

    def got3(r, c, g, m):
        sink(r, h + c, g, total((sg[4], m5[r, c, g]), (sg[2], m)))
        c22[r, c, g] = total((sg[2], m), (sg[0], m1[r, c, g]), (-sg[1], m2[r, c, g]))

    run(0, lambda r, c, g, m: m1.update({(r, c, g): m}))
    run(1, lambda r, c, g, m: m2.update({(r, c, g): m}))
    run(3, got4)
    run(4, lambda r, c, g, m: m5.update({(r, c, g): m}))
    run(2, got3)
    run(6, lambda r, c, g, m: sink(r, c, g, total((sg[6], m), (1, c11[r, c, g]), (-sg[4], m5[r, c, g]))))
    run(5, lambda r, c, g, m: sink(h + r, h + c, g, total((low * sg[5], m), (low, c22[r, c, g]))))


ROWS = (_flip(LHS_TERMS, True, False), RHS_TERMS, -1)
INNER = (_flip(LHS_TERMS, False, True), _flip(RHS_TERMS, True, False), 1)
KIND = [ROWS] * 3 + [INNER] * 5


def _tiles(sink, pre=lambda c, y: y):
    parts = {}

    def part(r, c, g, y):
        parts.setdefault((r, c), []).append(pre(c, y))
        if g == TPP - 1:
            y = jnp.concatenate(parts.pop((r, c)), axis=0)
            for t in range(2):
                sink(2 * c + t, r, y[:, 128 * t:128 * t + 128])
    return part


class _Side:
    def __init__(self, jobs, span, start=0, room=None):
        room = room[start:start + span] if room else [1] * span
        self.jobs, self.n, self.done = list(jobs), -start, 0
        self.due = [len(self.jobs) * sum(room[:k + 1]) // sum(room) for k in range(span)]

    def tick(self, fence):
        while 0 <= self.n < len(self.due) and self.done < self.due[self.n]:
            self.jobs[self.done](fence)
            self.done += 1
        self.n += 1


def _room(*busy):
    final = (2, 4, 5, 6)
    return [10] * FLAG + [b if o in final and i in final else R2 if i in final else 10
                          for b in busy for o in range(7) for i in range(7) for _ in range(TPP)]


def _staggered(gens, phases):
    def job(n):
        for k in reversed(range(phases)):
            if 0 <= n - k < len(gens):
                next(gens[n - k], None)
    return [lambda n=n: job(n) for n in range(len(gens) + phases - 1)]


def _run(jobs):
    for job in jobs:
        job(lambda ref: None)


def _kernel(x_hbm, wa_hbm, woa_hbm, wb_hbm, wob_hbm, out_hbm,
            wfa, wfb, af, woa, raw, xio, xr, st, oc, pv, kv, zs, zb, qT, kk, vT, sb, pc, sem):
    lane_head = lax.broadcasted_iota(jnp.int32, (128, 128), 1) // DH
    row_head = lax.broadcasted_iota(jnp.int32, (128, 128), 0) // DH
    same_head = lane_head == row_head
    on = lambda name: ONLY is None or name in ONLY
    RG = MQ // TPP
    wf = [(wfa, 0), (wfa, 1), (wfa, 2), (wfa, 3), (wfb, 0), (wfb, 1), (wfb, 2), (wfa, 4)]
    T7 = 7 * TPP
    st_fence, oc_fence = st.at[RB:RB + 8, 0:128], oc.at[32, 0:8, 0:128]

    def packed(ref, *idx):
        return pltpu.bitcast(ref.bitcast(u32)[idx], bf16)

    pending = []

    def tick(sides, done, g, y):
        fence = lambda ref: None
        if len(pending) >= FLAG:
            fn, g0, y0 = pending.pop(0)
            fn(g0, y0)

            def fence(ref):
                ref[...] = y0[0:ref.shape[0], 0:128].astype(ref.dtype)
        for side in sides:
            side.tick(fence)
        pending.append((done, g, y))

    def project(w, sides, sink):
        def prod(p, done):
            y = _dot(jnp.concatenate([packed(af, p, c) for c in range(2)], axis=1),
                     jnp.concatenate([packed(*wf[w], p, c) for c in range(2)], axis=1))
            for g in range(TPP):
                tick(sides, done, g, y[g * RG:(g + 1) * RG])
        _strassen(KIND[w], prod, sink)

    def drain():
        while pending:
            fn, g, y = pending.pop(0)
            fn(g, y)

    def fenced(ref, jobs):
        def run(fence, job):
            fence(ref)
            job()
        return [lambda fence, job=job: run(fence, job) for job in jobs]

    def at(r, c, g):
        return slice(r * MQ + g * RG, r * MQ + (g + 1) * RG), slice(c * KQ, (c + 1) * KQ)

    def blk(i):
        return pl.ds(pl.multiple_of(i * RB, RB), RB)

    def form_jobs(table, dst, tile, groups, rows):
        def halves(r, c, i):
            top = _forms(table, i, lambda a, b: tile(a, b, r, c))
            if HALF:
                yield
            for j, f in enumerate(_forms(table, i, lambda a, b: tile(a, b, r + 8, c))):
                dst[7 * i + j, c, r:r + 16, :] = jnp.concatenate([top[j], f], axis=0).astype(bf16)
        gens = [halves(r, c, i) for i in groups for r in range(0, rows, 16) for c in range(2)]
        if rows == 16:
            gens = gens[0::2] + gens[1::2]
        return [lambda g=g: next(g, None) for g in gens for _ in range(1 + HALF)]

    def lanes(b, c):
        return slice(b * KQ + 128 * c, b * KQ + 128 * c + 128)

    def lhs_jobs(w, b, groups):
        src = st.at[blk(b)]
        return fenced(st_fence, form_jobs(KIND[w][0], af, lambda a, b, r, c: src[a * MQ + r:a * MQ + r + 8, lanes(b, c)],
                                          groups, MQ))

    def operand_sides(w, w_next, fill, room, share):
        span = len(room) - FLAG
        per = int(min(T7, span * (1.0 - share) / 7))
        a, b = (7 - AHEAD) * per, span - AHEAD * per
        return [_Side(lhs_jobs(w, zero, ORDER[AHEAD:]), a, 0, room), _Side(fill, b - a - 4, a, room),
                _Side(lhs_jobs(w_next, zero, ORDER[:AHEAD]), span - b - 2, b, room)]

    raw_fence = raw.at[4 * D:4 * D + 16, 0:128]

    def raw_jobs(kind, dst, t, groups=ORDER, r0=0, rows=KQ):
        src = raw.at[pl.ds(pl.multiple_of(t * D + r0, 16), D - KQ + rows)]
        return fenced(raw_fence, form_jobs(kind[1], dst, lambda a, b, r, c: src[a * KQ + r:a * KQ + r + 8, lanes(b, c)].astype(f32),
                                           groups, rows))

    def norm_jobs(ref, i):
        x = lambda r: ref.at[blk(i)][r, :].astype(f32)

        def rows(r):
            mu = jnp.mean(x(r), axis=-1, keepdims=True)
            for _ in range(LN_GAP):
                yield
            xc = x(r) - mu
            rstd = lax.rsqrt(jnp.mean(xc * xc, axis=-1, keepdims=True) + 1e-5)
            for _ in range(LN_GAP):
                yield
            st[r, :] = (x(r) - mu) * rstd
        return fenced(ref.at[S:, 0:128],
                      _staggered([rows(slice(r, r + LN_ROWS)) for r in range(0, RB, LN_ROWS)], 2 * LN_GAP + 1))

    def front_jobs(denominator, i):
        def job(g, r):
            it, cols = i * NG + g, slice(r, r + 128)
            o = []
            for h in range(4):
                x = oc[it, DH * h:DH * h + DH, cols]
                o.append(x * (1.0 / denominator(x, g, it, h, cols)))
            st[r:r + 128, 128 * g:128 * g + 128] = jnp.concatenate(o, axis=0).T
        return fenced(oc_fence, [lambda g=g, r=r: job(g, r) for g in range(NG) for r in range(0, RB, 128)])

    def lin_den(x, g, it, h, cols):
        return jnp.sum(_fold8(None, x * zb[g, DH * h:DH * h + DH, :], jnp.add), axis=0, keepdims=True) + 1e-6

    def att_den(x, g, it, h, cols):
        return jnp.sum(oc[it, 128 + 8 * h:136 + 8 * h, cols], axis=0, keepdims=True)

    def out_copy(i):
        return pltpu.make_async_copy(xio.at[blk(i)], out_hbm.at[blk(i)], sem.at[i])

    def out_project(w, den, x, emit):
        def block(i, sides):
            def sink(r, c, g, y):
                y = x.at[blk(i)][at(r, c, g)].astype(f32) + y
                if emit:
                    xio.at[blk(i)][at(r, c, g)] = y.astype(bf16)
                else:
                    xr.at[blk(i)][at(r, c, g)] = y

            project(w, sides, sink)
            drain()
            if emit:
                out_copy(i).start()

        lax.fori_loop(0, NRB - 1, lambda i, c: block(i, operand_sides(w, w, front_jobs(den, i + 1), _room(RO), FS1)), None)
        sides = operand_sides(w, (w + 1) % 8, norm_jobs(xr, zero), _room(RO), FS2)
        block(zero + NRB - 1, sides[:1] if emit else sides)

    def qkv_a(i, mul):
        def phi_k(c, y):
            y = _phi(y)
            zs[:, c * KQ:(c + 1) * KQ] += _fold8(None, y, jnp.add)
            return y

        def got_k(g, r, y):
            pv[0, g, r] = y.T.astype(bf16)

        def got_v(r, c, g, y):
            for t in range(2):
                pv[1, 2 * c + t, r, g * RG:(g + 1) * RG, :] = y[:, 128 * t:128 * t + 128].astype(bf16)

        def got_q(g, r, y):
            oc[i * NG + g, 0:128, r * MQ:(r + 1) * MQ] = _phi(y.T)

        mul(W_AK, _tiles(got_k, phi_k))
        mul(W_AQ, _tiles(got_q))
        mul(W_AV, got_v)
        for g in range(NG):
            if g == NG // 2:
                drain()
            kv[g] += _dot(jnp.concatenate([packed(pv, 0, g, r) for r in range(4)], axis=1),
                          pltpu.bitcast(pv.bitcast(u32)[1, g].reshape(RB // 2, 128), bf16))

    def zero_stats():
        kv[...] = jnp.zeros_like(kv)
        zs[...] = jnp.zeros_like(zs)

    def x_copy(i):
        return pltpu.make_async_copy(x_hbm.at[blk(i)], xio.at[blk(i)], sem.at[i])

    def wa_copy(w, r, n, s):
        return pltpu.make_async_copy(wa_hbm.at[pl.ds(r, n), pl.ds(w * D, D)], raw.at[pl.ds((1 + w) * D + r, n)],
                                     sem.at[NRB + 5 + s])

    wk_cp = [[wa_copy(W_AK, a * KQ + r, n, 2 + 4 * t + a) for a in range(4)] for t, (r, n) in enumerate(WK_SPLIT)]
    wq_cp, wv_cp = wa_copy(W_AQ, 0, D, 0), wa_copy(W_AV, 0, D, 1)
    wb_cp = [pltpu.make_async_copy(a, raw.at[pl.ds(t * D, D)], sem.at[NRB + t])
             for t, a in enumerate([wb_hbm.at[:, pl.ds(c * D, D)] for c in range(3)] + [wob_hbm])]
    wo_cp = pltpu.make_async_copy(woa_hbm, woa, sem.at[NRB + 4])

    with jax.named_scope("s0"):
        for c in [x_copy(0)] + sum(wk_cp, []) + [wq_cp]:
            c.start()
        zero_stats()
        zero = lax.fori_loop(0, 2, lambda j, c: c + j // 8, 0)

    def sync(at, done, new):
        def job(fence):
            for c in done:
                c.wait()
            for c in new:
                c.start()
        return _Side([job], 1, at - 1)

    if on("p00"):
        x_copy(0).wait()
        x = xio[0:RB, :].astype(f32)
        x = x - jnp.mean(x, axis=-1, keepdims=True)
        st[0:RB, :] = x * lax.rsqrt(jnp.mean(x * x, axis=-1, keepdims=True) + 1e-5)
        _run(lhs_jobs(W_AQ, zero, ORDER[:AHEAD]))

        def prepare(w, cps, r0, n):
            def rows(j, c):
                r = pl.multiple_of(r0 + 16 * j, 16)
                _run(raw_jobs(ROWS, wfa.at[w, :, :, pl.ds(r, 16)], 1 + w, ORDER, r, 16))
            for c in cps:
                c.wait()
            lax.fori_loop(0, n // 16, rows, None)

        for cps, (r0, n) in zip(wk_cp, WK_SPLIT):
            prepare(W_AK, cps, r0, n)
        wv_cp.start()
        x_copy(1).start()
        room = _room(*RA)
        sides = [_Side(lhs_jobs(W_AQ, zero, ORDER[AHEAD:]), 4 * T7, 0, room),
                 _Side(raw_jobs(ROWS, wfa.at[W_AV], zero + 1 + W_AV), TC * TPP - 7 * T7, 7 * T7, room),
                 sync(TD * TPP, [x_copy(1)], [wb_cp[0], x_copy(2)]),
                 _Side(norm_jobs(xio, zero + 1), 19 * T7 - TD * TPP - 4, TD * TPP, room),
                 _Side(lhs_jobs(W_AQ, zero, ORDER[:AHEAD]), 2 * T7, 19 * T7, room)]

        def first_mul(w, sink):
            if w == W_AQ:
                drain()
                prepare(w, [wq_cp], 0, KQ)
                wv_cp.wait()
            project(w, sides, sink)

        with jax.named_scope("p00"):
            qkv_a(zero, first_mul)

    def layer(l):
        def block_a(i, c):
            sides = operand_sides(W_AQ, W_AQ, norm_jobs(xr if l else xio, jnp.minimum(i + 1, NRB - 1)), _room(*RA), 0.5)
            if l == 0:
                for n in range(1, NRB):
                    @pl.when(i == n)
                    def _():
                        for c in [[wb_cp[1], x_copy(3)], [wb_cp[2], wo_cp], [wb_cp[3]]][n - 1]:
                            c.start()
                        wb_cp[n - 1].wait()
                        if n + 1 < NRB:
                            x_copy(n + 1).wait()

                sides.append(_Side(raw_jobs(INNER, wfb.at[i - 1], i - 1), 21 * T7, 0, _room(*RA)))
            qkv_a(i, lambda w, sink: project(w, sides, sink))

        with jax.named_scope("p0"):
            if on("p0"): lax.fori_loop(1 - l, NRB, block_a, None)
        if l == 0:
            wo_cp.wait()
            wb_cp[3].wait()

        with jax.named_scope("p1"):
          if on("p1"):
            z = jnp.sum(zs[...], axis=0, keepdims=True)
            wp = []
            for g in range(NG):
                cs = slice(128 * g, 128 * g + 128)
                zb[g] = jnp.broadcast_to(z[:, cs], (128, 128)).T
                wp.append(_dot(jnp.where(same_head, kv[g], 0.0).astype(bf16), woa[cs, :]))
            wp = jnp.concatenate(wp, axis=0)
            for job in form_jobs(INNER[1], wfa.at[3], lambda a, b, r, c: wp[a * KQ + r:a * KQ + r + 8, lanes(b, c)], ORDER, KQ):
                job()
            _run(front_jobs(lin_den, 0) + lhs_jobs(W_AO, zero, ORDER[:AHEAD]))
            if l == 0:
                zero_stats()
        with jax.named_scope("p2a"):
            if on("p2a"): out_project(W_AO, lin_den, xr if l else xio, False)

        def qkv_b(i, c):
            def got_q(g, r, y):
                qT[i * NG + g, :, r * MQ:(r + 1) * MQ] = y.T.astype(bf16)

            def got_v(g, r, y):
                vT[g, i * 4 + r] = y.T.astype(bf16)

            def got_k(r, c, g, y):
                for t in range(2):
                    kk[2 * c + t, i * 4 + r, g * RG:(g + 1) * RG, :] = y[:, 128 * t:128 * t + 128].astype(bf16)

            sides = operand_sides(W_BQ, W_BQ, norm_jobs(xr, jnp.minimum(i + 1, NRB - 1)), _room(*RBB), 0.5)
            if l == 0:
                r0 = pl.multiple_of(i * (KQ // NRB), 16)
                sides.append(_Side(raw_jobs(INNER, wfa.at[4, :, :, pl.ds(r0, KQ // NRB)], 3, ORDER, r0, KQ // NRB), 14 * T7, 5 * T7, _room(*RBB)))
            project(W_BQ, sides, _tiles(got_q, lambda c, y: y * QSCALE))
            project(W_BV, sides, _tiles(got_v))
            project(W_BK, sides, got_k)
            drain()

        with jax.named_scope("p2b"):
            if on("p2b"): lax.fori_loop(0, NRB, qkv_b, None)

        zq = jnp.zeros((DH, QB), bf16)

        def qk(it, h, j):
            q = qT[it, DH * h:DH * h + DH, :]
            q = jnp.concatenate([q if a == h else zq for a in range(4)], axis=0)
            return _dot(kk[it % NG, j], q)

        def fin_max(m):
            return jnp.broadcast_to(jnp.max(m, axis=0, keepdims=True), (8, QB))

        def expo(x, m):
            return jnp.exp2(x.reshape(x.shape[0] // 8, 8, QB) - m[None]).reshape(x.shape[0], QB)

        G = 16
        bufs = [sb.at[zero], sb.at[1 - zero]]

        def attend(it, state, sides=(), last=False):
            m, mn, lsum, p = state
            for n in range(4 * NS):
                h, j = divmod(n, NS)
                t1, j1 = divmod(n + NS + 1, NS)
                t2, j2 = divmod(n + 1, NS)
                score, weigh = not last or t1 < 4, not last or t2 < 4
                if score:
                    s = qk(it + t1 // 4, t1 % 4, j1)
                o = _dot(vT[it % NG, j, DH * h:DH * h + DH, :], p)
                if j1 == 0:
                    ldone, lsum = lsum, None
                    if weigh:
                        m, mn = fin_max(mn), None
                pp = [None] * (KB // G)
                for g in range(KB // G):
                    if score:
                        sg = s[g * G:(g + 1) * G]
                        bufs[t1 % 2][j1 * KB + g * G:j1 * KB + g * G + G, :] = sg
                        mn = _fold8(mn, sg, jnp.maximum)
                    if weigh and g % 2 == 0:
                        for gg in (KB // G - 1 - g, KB // G - 2 - g):
                            pp[gg] = expo(bufs[t2 % 2][j2 * KB + gg * G:j2 * KB + gg * G + G, :], m)
                            lsum = _fold8(lsum, pp[gg], jnp.add)
                if weigh:
                    p = jnp.concatenate(pp, axis=0).astype(bf16)
                acc = (jnp.full((DH, QB), zero.astype(f32)) if j == 0 else acc) + o

                def fence(ref):
                    ref[...] = o[0:8, 0:128]
                for side in sides:
                    side.tick(fence)
                if j == NS - 1:
                    oc[it, DH * h:DH * h + DH, :] = acc
                    oc[it, 128 + 8 * h:136 + 8 * h, :] = ldone
            return m, mn, lsum, p

        with jax.named_scope("p3"):
          if on("p3"):
            mn = None
            for n in range(NS + 1):
                h, j = divmod(n, NS)
                s = qk(0, h, j)
                sb[h, j * KB:(j + 1) * KB, :] = s
                if n == NS:
                    m, mn = fin_max(mn), None
                mn = _fold8(mn, s, jnp.maximum)
            p = expo(sb[0, 0:KB, :], m)
            state = m, mn, _fold8(None, p, jnp.add), p.astype(bf16)
            head = 31 % ATT_U
            for it in range(head):
                state = attend(it, state)
            pc[...] = state[3]

            def items(i, carry):
                state = carry + (pc[...],)
                for u in range(ATT_U):
                    state = attend(head + i * ATT_U + u, state)
                pc[...] = state[3]
                return state[:3]

            state = lax.fori_loop(0, 31 // ATT_U, items, state[:3]) + (pc[...],)
            attend(31, state, [_Side(front_jobs(att_den, zero), 48), _Side(lhs_jobs(W_BO, zero, ORDER[:AHEAD]), 14, 49)], True)

        with jax.named_scope("p4a"):
            if on("p4a"): out_project(W_BO, att_den, xr, l == 1)

    for l in LAYERS:
        layer(l)
    with jax.named_scope('end'):
        for i in range(NRB):
            out_copy(i).wait()


@jax.jit
def pallas_interleave_layers__linear_attn_block__mha_block__prompt_kernel(
    A_x, A_wqkv, A_wo, B_x, B_wqkv, B_wo,
):
    del B_x
    assert A_x.shape == (1, S, D)
    out = pl.pallas_call(
        _kernel,
        name="fused",
        out_shape=jax.ShapeDtypeStruct((S, D), bf16),
        in_specs=[pl.BlockSpec(memory_space=pl.ANY)] * 5,
        out_specs=pl.BlockSpec(memory_space=pl.ANY),
        scratch_shapes=[
            pltpu.VMEM((5, NPROD, 2, KQ, 128), bf16),
            pltpu.VMEM((3, NPROD, 2, KQ, 128), bf16),
            pltpu.VMEM((NPROD, 2, MQ, 128), bf16),
            pltpu.VMEM((D, D), bf16),
            pltpu.VMEM((4 * D + 16, D), bf16),
            pltpu.VMEM((S + 16, D), bf16),
            pltpu.VMEM((S + 8, D), f32),
            pltpu.VMEM((RB + 8, D), f32),
            pltpu.VMEM((33, 160, QB), f32),
            pltpu.VMEM((2, NG, 4, 128, 128), bf16),
            pltpu.VMEM((NG, 128, 128), f32),
            pltpu.VMEM((8, D), f32),
            pltpu.VMEM((NG, 128, 128), f32),
            pltpu.VMEM((32, 128, QB), bf16),
            pltpu.VMEM((NG, NS, KB, 128), bf16),
            pltpu.VMEM((NG, NS, 128, KB), bf16),
            pltpu.VMEM((2, S, QB), f32),
            pltpu.VMEM((KB, QB), bf16),
            pltpu.SemaphoreType.DMA((NRB + 7 + 4 * len(WK_SPLIT),)),
        ],
        compiler_params=pltpu.CompilerParams(vmem_limit_bytes=126 * 2**20),
    )(A_x.reshape(S, D), A_wqkv, A_wo, B_wqkv, B_wo)
    return out.reshape(1, S, D)
```

```python
import math

import jax
import jax.numpy as jnp
from jax import lax
from jax.experimental import pallas as pl
from jax.experimental.pallas import tpu as pltpu

f32, bf16, u32 = jnp.float32, jnp.bfloat16, jnp.uint32

S, D, H, DH = 2048, 1024, 32, 32
NG = D // 128
QSCALE = math.log2(math.e) * DH ** -0.5

RB = 512
NRB = S // RB
MQ, KQ = RB // 4, D // 4
NPROD = 49
TPP = 4
RG = MQ // TPP
T7 = 7 * TPP
LAG = 4
AHEAD = 2
LN_ROWS, LN_GAP = 8, 4
WK_SPLIT = ((0, 128), (128, 80), (208, 48))

KB = 128
NS = S // KB
G = 16
NV = 3
JB = 4
U = 2
ONLY = None
LAYERS = (0, 1)

W_AQ, W_AK, W_AV, W_AO, W_BQ, W_BK, W_BV, W_BO = range(8)


def _tree(xs, op):
    while len(xs) > 1:
        xs = [op(xs[i], xs[i + 1]) if i + 1 < len(xs) else xs[i] for i in range(0, len(xs), 2)]
    return xs[0]


def _fold8(acc, x, op):
    x = _tree([x[i:i + 8] for i in range(0, x.shape[0], 8)], op)
    return x if acc is None else op(acc, x)


def _dot(a, b):
    return jnp.dot(a, b, preferred_element_type=f32)


def _packed(ref, *idx):
    return pltpu.bitcast(ref.bitcast(u32)[idx], bf16)


def _tile(c):
    return slice(128 * c, 128 * c + 128)


def _phi(t):
    return jnp.where(t > 0, t + 1.0, jnp.exp(t)) + 1e-6


_LHS = [[(1, 0, 0), (1, 1, 1)], [(1, 1, 0), (1, 1, 1)], [(1, 0, 0)], [(1, 1, 1)],
        [(1, 0, 0), (1, 0, 1)], [(1, 1, 0), (-1, 0, 0)], [(1, 0, 1), (-1, 1, 1)]]
_RHS = [[(1, 0, 0), (1, 1, 1)], [(1, 0, 0)], [(1, 0, 1), (-1, 1, 1)], [(1, 1, 0), (-1, 0, 0)],
        [(1, 1, 1)], [(1, 0, 0), (1, 0, 1)], [(1, 1, 0), (1, 1, 1)]]
ORDER = (0, 1, 3, 4, 2, 6, 5)


def _flip(table, rows, cols):
    return [[(s * (-1 if rows and r else 1) * (-1 if cols and c else 1), r, c) for s, r, c in t] for t in table]


ROWS = (_flip(_LHS, True, False), _RHS, -1)
INNER = (_flip(_LHS, False, True), _flip(_RHS, True, False), 1)
KIND = [ROWS] * 3 + [INNER] * 5


def _signed_sum(terms):
    s0, x = terms[0]
    for s, v in terms[1:]:
        x = x + v if s == s0 else x - v
    return s0, x


def _forms(table, i, block):
    q = {(r, c): _signed_sum([(s, block(2 * ro + r, 2 * co + c)) for s, ro, co in table[i]])[1]
         for r in range(2) for c in range(2)}
    return [_signed_sum([(s, q[r, c]) for s, r, c in t])[1] for t in table]


def _strassen(kind, prod, sink, lev=2, base=0):
    if lev == 0:
        return prod(base, lambda g, m: sink(0, 0, g, m))
    h = 2 ** (lev - 1)
    lhs, rhs, low = kind
    sg = [a[0][0] * b[0][0] for a, b in zip(lhs, rhs)]
    m1, m2, m5, c11, c22 = {}, {}, {}, {}, {}

    def total(*terms):
        s, x = _signed_sum(sorted(terms, key=lambda t: -t[0]))
        assert s > 0
        return x

    def got4(r, c, g, m):
        sink(h + r, c, g, total((low * sg[1], m2[r, c, g]), (low * sg[3], m)))
        c11[r, c, g] = total((sg[0], m1[r, c, g]), (sg[3], m))

    def got3(r, c, g, m):
        sink(r, h + c, g, total((sg[4], m5[r, c, g]), (sg[2], m)))
        c22[r, c, g] = total((sg[2], m), (sg[0], m1[r, c, g]), (-sg[1], m2[r, c, g]))

    got = [lambda r, c, g, m: m1.update({(r, c, g): m}),
           lambda r, c, g, m: m2.update({(r, c, g): m}),
           got3,
           got4,
           lambda r, c, g, m: m5.update({(r, c, g): m}),
           lambda r, c, g, m: sink(h + r, h + c, g, total((low * sg[5], m), (low, c22[r, c, g]))),
           lambda r, c, g, m: sink(r, c, g, total((sg[6], m), (1, c11[r, c, g]), (-sg[4], m5[r, c, g])))]
    for i in ORDER:
        _strassen(kind, prod, got[i], lev - 1, base + i * 7 ** (lev - 1))


def _by_tile(sink, pre=lambda c, y: y):
    parts = {}

    def part(r, c, g, y):
        parts.setdefault((r, c), []).append(pre(c, y))
        if g == TPP - 1:
            y = jnp.concatenate(parts.pop((r, c)), axis=0)
            for t in range(2):
                sink(2 * c + t, r, y[:, _tile(t)])
    return part


class _Side:
    def __init__(self, jobs, span, start=0, room=None):
        room = room[start:start + span] if room else [1] * span
        self.jobs, self.n, self.done, self.due, used = list(jobs), -start, 0, [], 0
        for r in room:
            used += r
            self.due.append(len(self.jobs) * used // sum(room))

    def tick(self, fence):
        while 0 <= self.n < len(self.due) and self.done < self.due[self.n]:
            self.jobs[self.done](fence)
            self.done += 1
        self.n += 1


def _room(*busy):
    final = (2, 4, 5, 6)
    return [10] * LAG + [b if o in final and i in final else 10
                         for b in busy for o in range(7) for i in range(7) for _ in range(TPP)]


def _staggered(gens, phases):
    def job(n):
        for k in reversed(range(phases)):
            if 0 <= n - k < len(gens):
                next(gens[n - k], None)
    return [lambda n=n: job(n) for n in range(len(gens) + phases - 1)]


def _fenced(ref, jobs):
    def run(fence, job):
        fence(ref)
        job()
    return [lambda fence, job=job: run(fence, job) for job in jobs]


def _run(jobs):
    for job in jobs:
        job(lambda ref: None)


def _kernel(x_hbm, wa_hbm, woa_hbm, wb_hbm, wob_hbm, out_hbm,
            wfa, wfb, af, woa, raw, xio, xr, st, oc, pv, kv, zs, zb, qT, kk, vT, pc, kf, kb0, kb1, sem, *sb):
    on = lambda name: ONLY is None or name in ONLY
    wf = [(wfa, 0), (wfa, 1), (wfa, 2), (wfa, 3), (wfb, 0), (wfb, 1), (wfb, 2), (wfa, 4)]
    room_a, room_b, room_o = _room(0, 0, 3), _room(0, 0, 3), _room(2)

    def blk(i):
        return pl.ds(pl.multiple_of(i * RB, RB), RB)

    def x_copy(i):
        return pltpu.make_async_copy(x_hbm.at[blk(i)], xio.at[blk(i)], sem.at[i])

    def out_copy(i):
        return pltpu.make_async_copy(xio.at[blk(i)], out_hbm.at[blk(i)], sem.at[i])

    def wa_copy(w, r, n, s):
        return pltpu.make_async_copy(wa_hbm.at[pl.ds(r, n), pl.ds(w * D, D)], raw.at[pl.ds((1 + w) * D + r, n)],
                                     sem.at[NRB + 5 + s])

    wk_cp = [[wa_copy(W_AK, a * KQ + r, n, 2 + 4 * t + a) for a in range(4)] for t, (r, n) in enumerate(WK_SPLIT)]
    wq_cp, wv_cp = wa_copy(W_AQ, 0, D, 0), wa_copy(W_AV, 0, D, 1)
    wb_cp = [pltpu.make_async_copy(a, raw.at[pl.ds(t * D, D)], sem.at[NRB + t])
             for t, a in enumerate([wb_hbm.at[:, pl.ds(c * D, D)] for c in range(3)] + [wob_hbm])]
    wo_cp = pltpu.make_async_copy(woa_hbm, woa, sem.at[NRB + 4])

    for c in [x_copy(0)] + sum(wk_cp, []) + [wq_cp]:
        c.start()
    zero = lax.fori_loop(0, 2, lambda j, c: c + j // 8, 0)

    pending = []

    def project(w, sides, sink):
        def prod(p, done):
            y = _dot(jnp.concatenate([_packed(af, p, c) for c in range(2)], axis=1),
                     jnp.concatenate([_packed(*wf[w], p, c) for c in range(2)], axis=1))
            for g in range(TPP):
                fence = lambda ref: None
                if len(pending) >= LAG:
                    fn, g0, y0 = pending.pop(0)
                    fn(g0, y0)

                    def fence(ref):
                        ref[...] = y0[0:ref.shape[0], 0:128].astype(ref.dtype)
                for side in sides:
                    side.tick(fence)
                pending.append((done, g, y[g * RG:(g + 1) * RG]))
        _strassen(KIND[w], prod, sink)

    def drain():
        while pending:
            fn, g, y = pending.pop(0)
            fn(g, y)

    def form_jobs(table, dst, src, pitch, groups, rows):
        def job(r, c, i):
            tile = lambda a, b: src[a * pitch + r:a * pitch + r + 16, _tile(2 * b + c)].astype(f32)
            for j, f in enumerate(_forms(table, i, tile)):
                dst[7 * i + j, c, r:r + 16, :] = f.astype(bf16)
        todo = [(r, c, i) for i in groups for r in range(0, rows, 16) for c in range(2)]
        return [lambda t=t: job(*t) for t in (sorted(todo) if rows == 16 else todo)]

    def lhs_jobs(w, groups):
        return _fenced(st.at[RB:, 0:128], form_jobs(KIND[w][0], af, st.at[blk(zero)], MQ, groups, MQ))

    def rhs_jobs(kind, dst, slot, r0=0, rows=KQ):
        src = raw.at[pl.ds(pl.multiple_of(slot * D + r0, 16), D - KQ + rows)]
        return _fenced(raw.at[4 * D:, 0:128], form_jobs(kind[1], dst, src, KQ, ORDER, rows))

    def operand_sides(w, w_next, fill, room, share):
        span = len(room) - LAG
        per = int(min(T7, span * (1.0 - share) / 7))
        a, b = (7 - AHEAD) * per, span - AHEAD * per
        return [_Side(lhs_jobs(w, ORDER[AHEAD:]), a, 0, room), _Side(fill, b - a - 4, a, room),
                _Side(lhs_jobs(w_next, ORDER[:AHEAD]), span - b - 2, b, room)]

    def norm_jobs(ref, i):
        src = ref.at[blk(i)]

        def rows(r):
            mu = jnp.mean(src[r, :].astype(f32), axis=-1, keepdims=True)
            for _ in range(LN_GAP):
                yield
            xc = src[r, :].astype(f32) - mu
            rstd = lax.rsqrt(jnp.mean(xc * xc, axis=-1, keepdims=True) + 1e-5)
            for _ in range(LN_GAP):
                yield
            st[r, :] = (src[r, :].astype(f32) - mu) * rstd
        return _fenced(ref.at[S:, 0:128],
                       _staggered([rows(slice(r, r + LN_ROWS)) for r in range(0, RB, LN_ROWS)], 2 * LN_GAP + 1))

    def head_jobs(denominator, i):
        def job(g, c):
            o = []
            for hd in range(4 * g, 4 * g + 4):
                x = oc[i, hd, 0:DH, _tile(c)]
                o.append(x * (1.0 / denominator(x, i, hd, c)))
            st[_tile(c), _tile(g)] = jnp.concatenate(o, axis=0).T
        return _fenced(oc.at[0, H, 0:8, 0:128], [lambda g=g, c=c: job(g, c) for g in range(NG) for c in range(4)])

    def linear_den(x, i, hd, c):
        return jnp.sum(_fold8(None, x * zb[DH * hd:DH * hd + DH, :], jnp.add), axis=0, keepdims=True) + 1e-6

    def softmax_den(x, i, hd, c):
        return jnp.sum(oc[i, hd, DH:DH + 8, _tile(c)], axis=0, keepdims=True)

    def out_project(w, den, x, final):
        def block(i, sides):
            src, dst = x.at[blk(i)], (xio if final else xr).at[blk(i)]

            def sink(r, c, g, y):
                at = slice(r * MQ + g * RG, r * MQ + (g + 1) * RG), slice(c * KQ, (c + 1) * KQ)
                dst[at] = (src[at].astype(f32) + y).astype(dst.dtype)

            project(w, sides, sink)
            drain()
            if final:
                out_copy(i).start()

        lax.fori_loop(0, NRB - 1, lambda i, c: block(i, operand_sides(w, w, head_jobs(den, i + 1), room_o, 0.45)), None)
        sides = operand_sides(w, (w + 1) % 8, norm_jobs(xr, zero), room_o, 0.55)
        block(zero + NRB - 1, sides[:1] if final else sides)

    def clear_summaries():
        kv[...] = jnp.zeros_like(kv)
        zs[...] = jnp.zeros_like(zs)

    def linear_block(i, mul):
        def phi_k(c, y):
            y = _phi(y)
            zs[:, c * KQ:(c + 1) * KQ] += _fold8(None, y, jnp.add)
            return y

        def got_k(g, r, y):
            pv[0, g, r] = y.T.astype(bf16)

        def got_q(g, r, y):
            y = _phi(y.T)
            for h in range(4):
                oc[i, 4 * g + h, 0:DH, _tile(r)] = y[DH * h:DH * h + DH]

        def got_v(r, c, g, y):
            for t in range(2):
                pv[1, 2 * c + t, r, g * RG:(g + 1) * RG, :] = y[:, _tile(t)].astype(bf16)

        mul(W_AK, _by_tile(got_k, phi_k))
        mul(W_AQ, _by_tile(got_q))
        mul(W_AV, got_v)
        for g in range(NG):
            if g == NG // 2:
                drain()
            kv[g] += _dot(jnp.concatenate([_packed(pv, 0, g, r) for r in range(4)], axis=1),
                          pltpu.bitcast(pv.bitcast(u32)[1, g].reshape(RB // 2, 128), bf16))

    def first_block():
        def prepare(w, copies, r0, n):
            def rows(j, c):
                r = pl.multiple_of(r0 + 16 * j, 16)
                _run(rhs_jobs(ROWS, wfa.at[w, :, :, pl.ds(r, 16)], 1 + w, r, 16))
            for c in copies:
                c.wait()
            lax.fori_loop(0, n // 16, rows, None)

        def more(fence):
            x_copy(1).wait()
            wb_cp[0].start()
            x_copy(2).start()

        def mul(w, sink):
            if w == W_AQ:
                drain()
                prepare(w, [wq_cp], 0, KQ)
                wv_cp.wait()
            project(w, sides, sink)

        x_copy(0).wait()
        x = xio[0:RB, :].astype(f32)
        x = x - jnp.mean(x, axis=-1, keepdims=True)
        st[0:RB, :] = x * lax.rsqrt(jnp.mean(x * x, axis=-1, keepdims=True) + 1e-5)
        _run(lhs_jobs(W_AQ, ORDER[:AHEAD]))
        for copies, (r0, n) in zip(wk_cp, WK_SPLIT):
            prepare(W_AK, copies, r0, n)
        wv_cp.start()
        x_copy(1).start()
        t = 64 * TPP
        sides = [_Side(lhs_jobs(W_AQ, ORDER[AHEAD:]), 4 * T7, 0, room_a),
                 _Side(rhs_jobs(ROWS, wfa.at[W_AV], zero + 1 + W_AV), 73 * TPP, 7 * T7, room_a),
                 _Side([more], 1, t - 1),
                 _Side(norm_jobs(xio, zero + 1), 19 * T7 - t - 4, t, room_a),
                 _Side(lhs_jobs(W_AQ, ORDER[:AHEAD]), 2 * T7, 19 * T7, room_a)]
        linear_block(zero, mul)

    def linear_attention(first):
        def block(i, c):
            fill = norm_jobs(xio if first else xr, jnp.minimum(i + 1, NRB - 1))
            sides = operand_sides(W_AQ, W_AQ, fill, room_a, 0.5)
            if first:
                for n in range(1, NRB):
                    @pl.when(i == n)
                    def _():
                        wb_cp[n].start()
                        if n + 1 < NRB:
                            (x_copy(3) if n == 1 else wo_cp).start()
                            x_copy(n + 1).wait()
                        wb_cp[n - 1].wait()

                sides.append(_Side(rhs_jobs(INNER, wfb.at[i - 1], i - 1), 21 * T7, 0, room_a))
            linear_block(i, lambda w, sink: project(w, sides, sink))

        if first and on("p00"):
            with jax.named_scope("p00"):
                first_block()
        with jax.named_scope("p0"):
            if on("p0"): lax.fori_loop(1 if first else 0, NRB, block, None)
        if first:
            wo_cp.wait()
            wb_cp[3].wait()

        with jax.named_scope("p1"):
          if on("p1"):
            same_head = (lax.broadcasted_iota(jnp.int32, (128, 128), 0) // DH
                         == lax.broadcasted_iota(jnp.int32, (128, 128), 1) // DH)
            z = jnp.sum(zs[...], axis=0, keepdims=True)
            folded = []
            for g in range(NG):
                zb[_tile(g), :] = jnp.broadcast_to(z[:, _tile(g)], (128, 128)).T
                folded.append(_dot(jnp.where(same_head, kv[g], 0.0).astype(bf16), woa[_tile(g), :]))
            for job in form_jobs(INNER[1], wfa.at[W_AO], jnp.concatenate(folded, axis=0), KQ, ORDER, KQ):
                job()
            _run(head_jobs(linear_den, 0) + lhs_jobs(W_AO, ORDER[:AHEAD]))
            if first:
                clear_summaries()
        with jax.named_scope("p2a"):
            if on("p2a"): out_project(W_AO, linear_den, xio if first else xr, False)

    half = [zero, 1 - zero]
    short = [NS * (t + 1) // NV - 1 for t in range(NV)]
    slots = [(j, g) for j in range(1, NS) for g in range(KB // G)][:-3]
    due = [(2 * NV * 4 * DH * k + len(slots)) // (2 * len(slots)) for k in range(len(slots) + 1)]
    terms = {slot: range(due[k], due[k + 1]) for k, slot in enumerate(slots)}
    wanted = {}
    for (j, g), us in terms.items():
        for u in us:
            wanted.setdefault((j // JB * 2 + g % 2, u // (NV * DH)), j)

    def scores(j, g, item):
        j = (j - (g == KB // G - 1)) % NS
        return sb[j // JB * 2 + g % 2].at[item, j % JB, g // 2 * G:g // 2 * G + G]

    def head_rows(hd, n):
        return pl.ds(pl.multiple_of(hd % 4 * n, n), n)

    def qk(hd, odd, i, j, rows=KB):
        q = jnp.concatenate([qT.bitcast(u32)[hd // 4, i, c, head_rows(hd, DH // 2)] for c in range(4)], axis=1)
        q = jnp.concatenate([q if a == odd else jnp.zeros_like(q) for a in range(4)], axis=0)
        return _dot(_packed(kk, hd // 2, j, slice(0, rows // 2)), pltpu.bitcast(q, bf16))

    def widen_q(hd, i, j):
        for (a, c), j0 in wanted.items():
            if j0 == j:
                sb[a][zero, JB, 0:DH, _tile(c)] = qT[hd // 4, i, c, head_rows(hd, DH), :].astype(f32)

    def key_jobs(hd, odd):
        def job(t, d):
            (kb0, kb1)[odd][0, t, d] = jnp.broadcast_to(kf[zero, t][:, odd * DH + d:odd * DH + d + 1], (G, 128))

        for t, j in enumerate(short):
            kf[0, t] = kk[hd // 2, j, KB - G:KB, :].astype(f32)
        return _fenced(kf.at[0, NV, 0:8], [lambda t=t, d=d: job(t, d) for d in range(DH) for t in range(NV)])

    def row_max(m):
        return jnp.broadcast_to(jnp.max(jnp.concatenate(m, axis=1), axis=0, keepdims=True), (8, RB))

    def fold_max(m, s):
        s = _fold8(None, s, jnp.maximum)
        return [s[:, _tile(c)] if x is None else jnp.maximum(x, s[:, _tile(c)]) for c, x in enumerate(m)]

    def weights(s, m):
        return jnp.exp2(s.reshape(s.shape[0] // 8, 8, RB) - m[None]).reshape(s.shape)

    def attend(hd, odd, state, sides=None):
        last = sides is not None
        sides = sides if last else [_Side(key_jobs(hd + 1, 1 - odd), 28 * 8, 2 * 8)]
        m, mn, lsum, p = state
        partial = []
        for n in range(NRB * NS):
            i, j = divmod(n, NS)
            t1, j1 = divmod(n + NS + 1, NS)
            t2, j2 = divmod(n + 1, NS)
            h1, odd1 = hd + t1 // NRB, (odd + t1 // NRB) % 2
            score, weigh, cut = not last or t1 < NRB, not last or t2 < NRB, j1 in short
            if score:
                widen_q(h1, t1 % NRB, j1 + 1)
                s = qk(h1, odd1, t1 % NRB, j1, KB - G if cut else KB)
            o = _dot(_packed(vT, hd // 4, j, head_rows(hd, DH // 2)), p)
            if j1 == 0:
                ldone, lsum = lsum, None
                if weigh:
                    m, mn = row_max(mn), [None] * 4
            pp = []
            for g in range(KB // G):
                mark = o
                if score:
                    near = sb[j1 // JB * 2 + g % 2]
                    for u in terms.get((j1, g), ()):
                        c, t, d = u // (NV * DH), u // DH % NV, u % DH
                        y = (kb0, kb1)[odd1][zero, t, d] * near[2 * zero, JB, d:d + 1, _tile(c)]
                        sv = y if d == 0 else sv + y
                        if d == DH - 1:
                            mn[c] = _fold8(mn[c], sv, jnp.maximum)
                            scores(short[t], KB // G - 1, half[t1 % 2])[:, _tile(c)] = sv
                    if (j1, g) in terms:
                        partial.append(sv)
                        if len(partial) == 2:
                            near[half[t1 % 2], JB, DH:DH + G, 0:128] = partial.pop(0)
                    if not (cut and g == KB // G - 1):
                        mark = s[g * G:(g + 1) * G]
                        scores(j1, g, half[t1 % 2])[...] = mark
                        mn = fold_max(mn, mark)

                def fence(ref):
                    ref[...] = mark[0:8, 0:128]
                for side in sides:
                    side.tick(fence)
                if weigh:
                    pp.insert(0, weights(scores(j2, KB // G - 1 - g, half[t2 % 2])[...], m))
                    lsum = _fold8(lsum, pp[0], jnp.add)
            if weigh:
                p = jnp.concatenate(pp, axis=0).astype(bf16)
            acc = (jnp.full((DH, RB), zero.astype(f32)) if j == 0 else acc) + o
            if j == NS - 1:
                oc[i, hd, 0:DH, :] = acc
                oc[i, hd, DH:DH + 8, :] = ldone
        return m, mn, lsum, p

    def softmax_attention(first):
        def block(i, c):
            def got_q(g, r, y):
                qT[g, i, r] = y.T.astype(bf16)

            def got_v(g, r, y):
                vT[g, i * 4 + r] = y.T.astype(bf16)

            def got_k(r, c, g, y):
                for t in range(2):
                    at = i * 4 + r, slice(g * RG, (g + 1) * RG)
                    kk[(4 * c + 2 * t,) + at] = y[:, _tile(t)].astype(bf16)
                    kk[(4 * c + 2 * t + 1,) + at] = pltpu.roll(y[:, _tile(t)], 2 * DH, 1).astype(bf16)

            sides = operand_sides(W_BQ, W_BQ, norm_jobs(xr, jnp.minimum(i + 1, NRB - 1)), room_b, 0.5)
            if first:
                n = KQ // NRB
                r0 = pl.multiple_of(i * n, 16)
                sides.append(_Side(rhs_jobs(INNER, wfa.at[4, :, :, pl.ds(r0, n)], 3, r0, n), 14 * T7, 5 * T7, room_b))
            project(W_BQ, sides, _by_tile(got_q, lambda c, y: y * QSCALE))
            project(W_BV, sides, _by_tile(got_v))
            project(W_BK, sides, got_k)
            drain()

        def park(state):
            for c in range(4):
                pc[c] = state[3][:, _tile(c)]
            return state[:3]

        def resume(carry):
            return carry + (jnp.concatenate([_packed(pc, c) for c in range(4)], axis=1),)

        def heads(i, carry):
            state = resume(carry)
            for u in range(U):
                state = attend(lead + U * i + u, (lead + u) % 2, state)
            return park(state)

        with jax.named_scope("p2b"):
            if on("p2b"): lax.fori_loop(0, NRB, block, None)
        with jax.named_scope("p3"):
          if on("p3"):
            _run(key_jobs(0, 0))
            widen_q(0, 1, 1)
            mn = [None] * 4
            for n in range(NS + 1):
                i, j = divmod(n, NS)
                s = qk(0, 0, i, j)
                for g in range(KB // G):
                    scores(j, g, i)[...] = s[g * G:(g + 1) * G]
                if n == NS:
                    m, mn = row_max(mn), [None] * 4
                mn = fold_max(mn, s)
            p = weights(jnp.concatenate([scores(0, g, 0)[...] for g in range(KB // G)], axis=0), m)
            state = m, mn, _fold8(None, p, jnp.add), p.astype(bf16)
            lead = (H - 1) % U
            for hd in range(lead):
                state = attend(hd, hd % 2, state)
            state = resume(lax.fori_loop(0, (H - 1) // U, heads, park(state)))
            attend(H - 1, 1, state, [_Side(head_jobs(softmax_den, zero), 48 * 8),
                                     _Side(lhs_jobs(W_BO, ORDER[:AHEAD]), 14 * 8, 49 * 8)])
        with jax.named_scope("p4a"):
            if on("p4a"): out_project(W_BO, softmax_den, xr, not first)

    clear_summaries()
    for layer in LAYERS:
        linear_attention(layer == 0)
        softmax_attention(layer == 0)
    for i in range(NRB):
        out_copy(i).wait()


@jax.jit
def pallas_interleave_layers__linear_attn_block__mha_block__prompt_kernel(
    A_x: jax.Array,
    A_wqkv: jax.Array,
    A_wo: jax.Array,
    B_x: jax.Array,
    B_wqkv: jax.Array,
    B_wo: jax.Array,
):
    del B_x
    assert A_x.shape == (1, S, D)
    out = pl.pallas_call(
        _kernel,
        name="fused",
        out_shape=jax.ShapeDtypeStruct((S, D), bf16),
        in_specs=[pl.BlockSpec(memory_space=pl.ANY)] * 5,
        out_specs=pl.BlockSpec(memory_space=pl.ANY),
        scratch_shapes=[
            pltpu.VMEM((5, NPROD, 2, KQ, 128), bf16),
            pltpu.VMEM((3, NPROD, 2, KQ, 128), bf16),
            pltpu.VMEM((NPROD, 2, MQ, 128), bf16),
            pltpu.VMEM((D, D), bf16),
            pltpu.VMEM((4 * D + 16, D), bf16),
            pltpu.VMEM((S + 16, D), bf16),
            pltpu.VMEM((S + 8, D), f32),
            pltpu.VMEM((RB + 8, D), f32),
            pltpu.VMEM((NRB, H + 1, DH + 8, RB), f32),
            pltpu.VMEM((2, NG, 4, 128, 128), bf16),
            pltpu.VMEM((NG, 128, 128), f32),
            pltpu.VMEM((8, D), f32),
            pltpu.VMEM((D, 128), f32),
            pltpu.VMEM((NG, NRB, 4, 128, 128), bf16),
            pltpu.VMEM((H // 2, NS, KB, 128), bf16),
            pltpu.VMEM((NG, NS, 128, KB), bf16),
            pltpu.VMEM((4, KB, 128), bf16),
            pltpu.VMEM((1, 2 * (NV // 2 + 1), G, 128), f32),
            pltpu.VMEM((1, NV, DH, G, 128), f32),
            pltpu.VMEM((1, NV, DH, G, 128), f32),
            pltpu.SemaphoreType.DMA((NRB + 7 + 4 * len(WK_SPLIT),)),
        ] + [pltpu.VMEM((2, JB + 1, KB // 2, RB), f32)] * (2 * NS // JB),
        compiler_params=pltpu.CompilerParams(vmem_limit_bytes=126 * 2**20),
    )(A_x.reshape(S, D), A_wqkv, A_wo, B_wqkv, B_wo)
    return out.reshape(1, S, D)
```

```python
import math

import jax
import jax.numpy as jnp
from jax import lax
from jax.experimental import pallas as pl
from jax.experimental.pallas import tpu as pltpu

f32, bf16, u32 = jnp.float32, jnp.bfloat16, jnp.uint32

S, D, H, DH = 2048, 1024, 32, 32
NG = D // 128
QSCALE = math.log2(math.e) * DH ** -0.5

RB = 512
NRB = S // RB
MQ, KQ = RB // 4, D // 4
NPROD = 49
TPP = 4
RG = MQ // TPP
T7 = 7 * TPP
LAG = 4
AHEAD = 2
LN_ROWS, LN_GAP = 8, 4
WK_SPLIT = ((0, 128), (128, 80), (208, 48))

KB = 128
NS = S // KB
G = 16
NV = 3
JB = 4

W_AQ, W_AK, W_AV, W_AO, W_BQ, W_BK, W_BV, W_BO = range(8)


def _tree(xs, op):
    while len(xs) > 1:
        xs = [op(xs[i], xs[i + 1]) if i + 1 < len(xs) else xs[i] for i in range(0, len(xs), 2)]
    return xs[0]


def _fold8(acc, x, op):
    x = _tree([x[i:i + 8] for i in range(0, x.shape[0], 8)], op)
    return x if acc is None else op(acc, x)


def _dot(a, b):
    return jnp.dot(a, b, preferred_element_type=f32)


def _packed(ref, *idx):
    return pltpu.bitcast(ref.bitcast(u32)[idx], bf16)


def _tile(c):
    return slice(128 * c, 128 * c + 128)


def _phi(t):
    return jnp.where(t > 0, t + 1.0, jnp.exp(t)) + 1e-6


_LHS = [[(1, 0, 0), (1, 1, 1)], [(1, 1, 0), (1, 1, 1)], [(1, 0, 0)], [(1, 1, 1)],
        [(1, 0, 0), (1, 0, 1)], [(1, 1, 0), (-1, 0, 0)], [(1, 0, 1), (-1, 1, 1)]]
_RHS = [[(1, 0, 0), (1, 1, 1)], [(1, 0, 0)], [(1, 0, 1), (-1, 1, 1)], [(1, 1, 0), (-1, 0, 0)],
        [(1, 1, 1)], [(1, 0, 0), (1, 0, 1)], [(1, 1, 0), (1, 1, 1)]]
ORDER = (0, 1, 3, 4, 2, 6, 5)


def _flip(table, rows, cols):
    return [[(s * (-1 if rows and r else 1) * (-1 if cols and c else 1), r, c) for s, r, c in t] for t in table]


ROWS = (_flip(_LHS, True, False), _RHS, -1)
INNER = (_flip(_LHS, False, True), _flip(_RHS, True, False), 1)
KIND = [ROWS] * 3 + [INNER] * 5


def _signed_sum(terms):
    s0, x = terms[0]
    for s, v in terms[1:]:
        x = x + v if s == s0 else x - v
    return s0, x


def _forms(table, i, block):
    q = {(r, c): _signed_sum([(s, block(2 * ro + r, 2 * co + c)) for s, ro, co in table[i]])[1]
         for r in range(2) for c in range(2)}
    return [_signed_sum([(s, q[r, c]) for s, r, c in t])[1] for t in table]


def _strassen(kind, prod, sink, lev=2, base=0):
    if lev == 0:
        return prod(base, lambda g, m: sink(0, 0, g, m))
    h = 2 ** (lev - 1)
    lhs, rhs, low = kind
    sg = [a[0][0] * b[0][0] for a, b in zip(lhs, rhs)]
    m1, m2, m5, c11, c22 = {}, {}, {}, {}, {}

    def total(*terms):
        s, x = _signed_sum(sorted(terms, key=lambda t: -t[0]))
        assert s > 0
        return x

    def got4(r, c, g, m):
        sink(h + r, c, g, total((low * sg[1], m2[r, c, g]), (low * sg[3], m)))
        c11[r, c, g] = total((sg[0], m1[r, c, g]), (sg[3], m))

    def got3(r, c, g, m):
        sink(r, h + c, g, total((sg[4], m5[r, c, g]), (sg[2], m)))
        c22[r, c, g] = total((sg[2], m), (sg[0], m1[r, c, g]), (-sg[1], m2[r, c, g]))

    got = [lambda r, c, g, m: m1.update({(r, c, g): m}),
           lambda r, c, g, m: m2.update({(r, c, g): m}),
           got3,
           got4,
           lambda r, c, g, m: m5.update({(r, c, g): m}),
           lambda r, c, g, m: sink(h + r, h + c, g, total((low * sg[5], m), (low, c22[r, c, g]))),
           lambda r, c, g, m: sink(r, c, g, total((sg[6], m), (1, c11[r, c, g]), (-sg[4], m5[r, c, g])))]
    for i in ORDER:
        _strassen(kind, prod, got[i], lev - 1, base + i * 7 ** (lev - 1))


def _by_tile(sink, pre=lambda c, y: y):
    parts = {}

    def part(r, c, g, y):
        parts.setdefault((r, c), []).append(pre(c, y))
        if g == TPP - 1:
            y = jnp.concatenate(parts.pop((r, c)), axis=0)
            for t in range(2):
                sink(2 * c + t, r, y[:, _tile(t)])
    return part


class _Side:
    def __init__(self, jobs, span, start=0, room=None):
        room = room[start:start + span] if room else [1] * span
        self.jobs, self.n, self.done, self.due, used = list(jobs), -start, 0, [], 0
        for r in room:
            used += r
            self.due.append(len(self.jobs) * used // sum(room))

    def tick(self, fence):
        while 0 <= self.n < len(self.due) and self.done < self.due[self.n]:
            self.jobs[self.done](fence)
            self.done += 1
        self.n += 1


def _room(*busy):
    final = (2, 4, 5, 6)
    return [10] * LAG + [b if o in final and i in final else 10
                         for b in busy for o in range(7) for i in range(7) for _ in range(TPP)]


def _staggered(gens, phases):
    def job(n):
        for k in reversed(range(phases)):
            if 0 <= n - k < len(gens):
                next(gens[n - k], None)
    return [lambda n=n: job(n) for n in range(len(gens) + phases - 1)]


def _fence(at, y):
    ref, rows = at[0], at[-1]
    ref[at[1:] + (slice(0, 128),)] = y[0:rows.stop - rows.start, 0:128].astype(ref.dtype)


def _fenced(at, jobs):
    def run(fence, job):
        fence(at)
        job()
    return [lambda fence, job=job: run(fence, job) for job in jobs]


def _run(jobs):
    for job in jobs:
        job(lambda at: None)


def _kernel(x_hbm, wa_hbm, woa_hbm, wb_hbm, wob_hbm, out_hbm,
            wfa, wfb, af, woa, raw, xio, xr, st, oc, pv, kv, zs, zb, qT, kk, vT, pc, kf, kb0, kb1, sem, *sb):
    wf = [(wfa, 0), (wfa, 1), (wfa, 2), (wfa, 3), (wfb, 0), (wfb, 1), (wfb, 2), (wfa, 4)]
    room_a, room_b, room_o = _room(0, 0, 1), _room(0, 0, 3), _room(1)

    def blk(i):
        return pl.ds(pl.multiple_of(i * RB, RB), RB)

    def x_copy(i):
        return pltpu.make_async_copy(x_hbm.at[blk(i)], xio.at[blk(i)], sem.at[i])

    def out_copy(i):
        return pltpu.make_async_copy(xio.at[blk(i)], out_hbm.at[blk(i)], sem.at[i])

    def wa_copy(w, r, n, s):
        return pltpu.make_async_copy(wa_hbm.at[pl.ds(r, n), pl.ds(w * D, D)], raw.at[pl.ds((1 + w) * D + r, n)],
                                     sem.at[NRB + 5 + s])

    wk_cp = [[wa_copy(W_AK, a * KQ + r, n, 2 + 4 * t + a) for a in range(4)] for t, (r, n) in enumerate(WK_SPLIT)]
    wq_cp, wv_cp = wa_copy(W_AQ, 0, D, 0), wa_copy(W_AV, 0, D, 1)
    wb_cp = [pltpu.make_async_copy(a, raw.at[pl.ds(t * D, D)], sem.at[NRB + t])
             for t, a in enumerate([wb_hbm.at[:, pl.ds(c * D, D)] for c in range(3)] + [wob_hbm])]
    wo_cp = pltpu.make_async_copy(woa_hbm, woa, sem.at[NRB + 4])
    corner = lambda ref, r, c: ref.at[pl.ds(S - RB + r * RB // 2, RB // 2), pl.ds(c * D // 2, D // 2)]
    tail_cp = [[pltpu.make_async_copy(corner(xio, r, c), corner(out_hbm, r, c), sem.at[NRB + 2 * r + c])
                for c in range(2)] for r in range(2)]

    for c in [x_copy(0)] + sum(wk_cp, []) + [wq_cp]:
        c.start()
    zero = lax.fori_loop(0, 2, lambda j, c: c + j // 8, 0)

    pending = []

    def project(w, sides, sink):
        def prod(p, done):
            y = _dot(jnp.concatenate([_packed(af, p, c) for c in range(2)], axis=1),
                     jnp.concatenate([_packed(*wf[w], p, c) for c in range(2)], axis=1))
            for g in range(TPP):
                fence = lambda at: None
                if len(pending) >= LAG:
                    fn, g0, y0 = pending.pop(0)
                    fn(g0, y0)

                    fence = lambda at: _fence(at, y0)
                for side in sides:
                    side.tick(fence)
                pending.append((done, g, y[g * RG:(g + 1) * RG]))
        _strassen(KIND[w], prod, sink)

    def drain():
        while pending:
            fn, g, y = pending.pop(0)
            fn(g, y)

    def form_jobs(table, dst, src, pitch, groups, rows):
        def job(r, c, i):
            tile = lambda a, b: src[a * pitch + r:a * pitch + r + 16, _tile(2 * b + c)].astype(f32)
            for j, f in enumerate(_forms(table, i, tile)):
                dst[7 * i + j, c, r:r + 16, :] = f.astype(bf16)
        todo = [(r, c, i) for i in groups for r in range(0, rows, 16) for c in range(2)]
        return [lambda t=t: job(*t) for t in (sorted(todo) if rows == 16 else todo)]

    def lhs_jobs(w, groups):
        return _fenced((st, slice(RB, RB + 8)), form_jobs(KIND[w][0], af, st.at[blk(zero)], MQ, groups, MQ))

    def rhs_jobs(kind, dst, slot, r0=0, rows=KQ):
        src = raw.at[pl.ds(pl.multiple_of(slot * D + r0, 16), D - KQ + rows)]
        return _fenced((raw, slice(4 * D, 4 * D + 16)), form_jobs(kind[1], dst, src, KQ, ORDER, rows))

    def operand_sides(w, w_next, fill, room, share):
        span = len(room) - LAG
        per = int(min(T7, span * (1.0 - share) / 7))
        a, b = (7 - AHEAD) * per, span - AHEAD * per
        return [_Side(lhs_jobs(w, ORDER[AHEAD:]), a, 0, room), _Side(fill, b - a - 4, a, room),
                _Side(lhs_jobs(w_next, ORDER[:AHEAD]), span - b - 2, b, room)]

    def norm_jobs(ref, i):
        src = ref.at[blk(i)]

        def rows(r):
            mu = jnp.mean(src[r, :].astype(f32), axis=-1, keepdims=True)
            for _ in range(LN_GAP):
                yield
            xc = src[r, :].astype(f32) - mu
            rstd = lax.rsqrt(jnp.mean(xc * xc, axis=-1, keepdims=True) + 1e-5)
            for _ in range(LN_GAP):
                yield
            st[r, :] = (src[r, :].astype(f32) - mu) * rstd
        return _fenced((ref, slice(S, ref.shape[0])),
                       _staggered([rows(slice(r, r + LN_ROWS)) for r in range(0, RB, LN_ROWS)], 2 * LN_GAP + 1))

    def head_jobs(denominator, i):
        def job(g, c):
            o = []
            for hd in range(4 * g, 4 * g + 4):
                x = oc[i, hd, 0:DH, _tile(c)]
                o.append(x * pltpu.reciprocal(denominator(x, i, hd, c), full_range=False))
            st[_tile(c), _tile(g)] = jnp.concatenate(o, axis=0).T
        return _fenced((oc, 0, H, slice(0, 8)), [lambda g=g, c=c: job(g, c) for g in range(NG) for c in range(4)])

    def linear_den(x, i, hd, c):
        return jnp.sum(_fold8(None, x * zb[DH * hd:DH * hd + DH, :], jnp.add), axis=0, keepdims=True) + 1e-6

    def softmax_den(x, i, hd, c):
        return jnp.sum(oc[i, hd, DH:DH + 8, _tile(c)], axis=0, keepdims=True)

    def out_project(w, den, x, final):
        def block(i, sides, last=False):
            src, dst = x.at[blk(i)], (xio if final else xr).at[blk(i)]

            def sink(r, c, g, y):
                at = slice(r * MQ + g * RG, r * MQ + (g + 1) * RG), slice(c * KQ, (c + 1) * KQ)
                dst[at] = (src[at].astype(f32) + y).astype(dst.dtype)
                if last and (r % 2, c % 2, g) == (1, 1, TPP - 1):
                    tail_cp[r // 2][c // 2].start()

            project(w, sides, sink)
            drain()
            if final and not last:
                out_copy(i).start()

        lax.fori_loop(0, NRB - 1, lambda i, c: block(i, operand_sides(w, w, head_jobs(den, i + 1), room_o, 0.4)), None)
        sides = operand_sides(w, (w + 1) % 8, norm_jobs(xr, zero), room_o, 0.55)
        if w == W_BO and not final:
            clear_summaries()
        block(zero + NRB - 1, sides[:1] if final else sides, final)

    def clear_summaries():
        kv[...] = jnp.zeros_like(kv)
        zs[...] = jnp.zeros_like(zs)

    def linear_block(i, mul):
        def phi_k(c, y):
            y = _phi(y)
            zs[:, c * KQ:(c + 1) * KQ] += _fold8(None, y, jnp.add)
            return y

        def got_k(g, r, y):
            pv[0, g, r] = y.T.astype(bf16)

        def got_q(g, r, y):
            y = _phi(y.T)
            for h in range(4):
                oc[i, 4 * g + h, 0:DH, _tile(r)] = y[DH * h:DH * h + DH]

        def got_v(r, c, g, y):
            for t in range(2):
                pv[1, 2 * c + t, r, g * RG:(g + 1) * RG, :] = y[:, _tile(t)].astype(bf16)

        mul(W_AK, _by_tile(got_k, phi_k))
        mul(W_AQ, _by_tile(got_q))
        mul(W_AV, got_v)
        for g in range(NG):
            if g == NG // 2:
                drain()
            kv[g] += _dot(jnp.concatenate([_packed(pv, 0, g, r) for r in range(4)], axis=1),
                          pltpu.bitcast(pv.bitcast(u32)[1, g].reshape(RB // 2, 128), bf16))

    def first_block():
        def prepare(w, copies, r0, n):
            def rows(j, c):
                r = pl.multiple_of(r0 + 16 * j, 16)
                _run(rhs_jobs(ROWS, wfa.at[w, :, :, pl.ds(r, 16)], 1 + w, r, 16))
            for c in copies:
                c.wait()
            lax.fori_loop(0, n // 16, rows, None)

        def more(fence):
            x_copy(1).wait()
            wb_cp[0].start()
            x_copy(2).start()

        def mul(w, sink):
            if w == W_AQ:
                drain()
                prepare(w, [wq_cp], 0, KQ)
                wv_cp.wait()
            project(w, sides, sink)

        x_copy(0).wait()
        x = xio[0:RB, :].astype(f32)
        x = x - jnp.mean(x, axis=-1, keepdims=True)
        st[0:RB, :] = x * lax.rsqrt(jnp.mean(x * x, axis=-1, keepdims=True) + 1e-5)
        _run(lhs_jobs(W_AQ, ORDER[:AHEAD]))
        for copies, (r0, n) in zip(wk_cp, WK_SPLIT):
            prepare(W_AK, copies, r0, n)
        wv_cp.start()
        x_copy(1).start()
        t = 64 * TPP
        sides = [_Side(lhs_jobs(W_AQ, ORDER[AHEAD:]), 4 * T7, 0, room_a),
                 _Side(rhs_jobs(ROWS, wfa.at[W_AV], zero + 1 + W_AV), 73 * TPP, 7 * T7, room_a),
                 _Side([more], 1, t - 1),
                 _Side(norm_jobs(xio, zero + 1), 19 * T7 - t - 4, t, room_a),
                 _Side(lhs_jobs(W_AQ, ORDER[:AHEAD]), 2 * T7, 19 * T7, room_a)]
        linear_block(zero, mul)

    def linear_attention(first):
        def block(i, c):
            fill = norm_jobs(xio if first else xr, jnp.minimum(i + 1, NRB - 1))
            sides = operand_sides(W_AQ, W_AQ, fill, room_a, 0.5)
            if first:
                for n in range(1, NRB):
                    @pl.when(i == n)
                    def _():
                        wb_cp[n].start()
                        if n + 1 < NRB:
                            (x_copy(3) if n == 1 else wo_cp).start()
                            x_copy(n + 1).wait()
                        wb_cp[n - 1].wait()

                sides.append(_Side(rhs_jobs(INNER, wfb.at[i - 1], i - 1), 21 * T7, 0, room_a))
            linear_block(i, lambda w, sink: project(w, sides, sink))

        if first:
            first_block()
        lax.fori_loop(1 if first else 0, NRB, block, None)
        if first:
            wo_cp.wait()
            wb_cp[3].wait()

        z = jnp.sum(zs[...], axis=0, keepdims=True)
        for g in range(NG):
            zb[_tile(g), :] = jnp.broadcast_to(z[:, _tile(g)], (128, 128)).T
        own = lax.broadcasted_iota(jnp.int32, (16, 128), 1) < DH
        sides = [_Side(head_jobs(linear_den, zero), 24), _Side(lhs_jobs(W_AO, ORDER[:AHEAD]), 8, 24)]
        for r in range(0, KQ, 16):
            rows = []
            for a in range(4):
                g, r0 = divmod(a * KQ + r, 128)
                shift = -(r0 // DH * DH) % 128
                y = kv[g, r0:r0 + 16, :]
                rows.append(jnp.where(own, pltpu.roll(y, shift, 1) if shift else y, 0.0).astype(bf16))
            for c in range(2):
                folded = []
                for a in range(4):
                    k = (a * KQ + r) // DH * DH
                    w = jnp.concatenate([woa[k:k + DH, _tile(2 * b + c)] for b in range(4)], axis=1)
                    folded.append(_dot(rows[a], jnp.concatenate([w, jnp.zeros((128 - DH, 512), bf16)], axis=0)))
                for i in range(7):
                    for j, f in enumerate(_forms(INNER[1], i, lambda a, b: folded[a][:, _tile(b)])):
                        wfa[W_AO, 7 * i + j, c, r:r + 16, :] = f.astype(bf16)
                for side in sides:
                    side.tick(lambda at: _fence(at, folded[0]))
        out_project(W_AO, linear_den, xio if first else xr, False)

    half, also_zero = [zero, 1 - zero], 2 * zero
    short = [NS * (t + 1) // NV - 1 for t in range(NV)]
    slots = [(j, g) for j in range(1, NS) for g in range(KB // G)][:-3]
    due = [(2 * NV * 4 * DH * k + len(slots)) // (2 * len(slots)) for k in range(len(slots) + 1)]
    terms = {slot: range(due[k], due[k + 1]) for k, slot in enumerate(slots)}
    wanted = {}
    for (j, g), us in terms.items():
        for u in us:
            wanted.setdefault((j // JB * 2 + g % 2, u // (NV * DH)), j)

    def scores(j, g, item, cols=slice(None)):
        j = (j - (g == KB // G - 1)) % NS
        return sb[j // JB * 2 + g % 2], (item, j % JB, slice(g // 2 * G, g // 2 * G + G), cols)

    def put_scores(s, *where):
        ref, idx = scores(*where)
        ref[idx] = s

    def get_scores(*where):
        ref, idx = scores(*where)
        return ref[idx]

    def head(hd, odd):
        rows = lambda n: pl.ds(pl.multiple_of((hd & 3) * n, n), n)
        return hd, odd, hd >> 1, hd >> 2, rows(DH), rows(DH // 2)

    def qk(h, i, j, rows=KB):
        q = jnp.concatenate([qT.bitcast(u32)[h[3], i, c, h[5]] for c in range(4)], axis=1)
        q = jnp.concatenate([q if a == h[1] else jnp.zeros_like(q) for a in range(4)], axis=0)
        return _dot(_packed(kk, h[2], j, slice(0, rows // 2)), pltpu.bitcast(q, bf16))

    def widen_q(h, i, j):
        for (a, c), j0 in wanted.items():
            if j0 == j:
                sb[a][zero, JB, 0:DH, _tile(c)] = qT[h[3], i, c, h[4], :].astype(f32)

    def key_jobs(h):
        def job(t, d):
            lane = h[1] * DH + d
            (kb0, kb1)[h[1]][0, t, d] = jnp.broadcast_to(kf[zero, t][:, lane:lane + 1], (G, 128))

        for t, j in enumerate(short):
            kf[0, t] = kk[h[2], j, KB - G:KB, :].astype(f32)
        return _fenced((kf, 0, NV, slice(0, 8)), [lambda t=t, d=d: job(t, d) for d in range(DH) for t in range(NV)])

    def row_max(m):
        return jnp.broadcast_to(jnp.max(jnp.concatenate(m, axis=1), axis=0, keepdims=True), (8, RB))

    def fold_max(m, s):
        s = _fold8(None, s, jnp.maximum)
        return [s[:, _tile(c)] if x is None else jnp.maximum(x, s[:, _tile(c)]) for c, x in enumerate(m)]

    def weights(s, m):
        return jnp.exp2(s.reshape(s.shape[0] // 8, 8, RB) - m[None]).reshape(s.shape)

    def attend(hd, odd, state, sides=None):
        last = sides is not None
        this, nxt = head(hd, odd), head(hd + 1, 1 - odd)
        sides = sides if last else [_Side(key_jobs(nxt), 28 * 8, 2 * 8)]
        m, mn, lsum, p = state
        partial, nothing = [], jnp.full((DH, RB), zero.astype(f32))
        for n in range(NRB * NS):
            i, j = divmod(n, NS)
            t1, j1 = divmod(n + NS + 1, NS)
            t2, j2 = divmod(n + 1, NS)
            h1 = this if t1 < NRB else nxt
            score, weigh, cut = not last or t1 < NRB, not last or t2 < NRB, j1 in short
            if score:
                widen_q(h1, t1 % NRB, j1 + 1)
                s = qk(h1, t1 % NRB, j1, KB - G if cut else KB)
            o = _dot(_packed(vT, this[3], j, this[5]), p)
            if j1 == 0:
                ldone, lsum = lsum, None
                if weigh:
                    m, mn = row_max(mn), [None] * 4
            pp = []
            for g in range(KB // G):
                mark = o
                if score:
                    near = sb[j1 // JB * 2 + g % 2]
                    for u in terms.get((j1, g), ()):
                        c, t, d = u // (NV * DH), u // DH % NV, u % DH
                        y = (kb0, kb1)[h1[1]][zero, t, d] * near[also_zero, JB, d:d + 1, _tile(c)]
                        sv = y if d == 0 else sv + y
                        if d == DH - 1:
                            mn[c] = _fold8(mn[c], sv, jnp.maximum)
                            put_scores(sv, short[t], KB // G - 1, half[t1 % 2], _tile(c))
                    if (j1, g) in terms:
                        partial.append(sv)
                        if len(partial) == 2:
                            near[half[t1 % 2], JB, DH:DH + G, 0:128] = partial.pop(0)
                    if not (cut and g == KB // G - 1):
                        mark = s[g * G:(g + 1) * G]
                        put_scores(mark, j1, g, half[t1 % 2])
                        mn = fold_max(mn, mark)
                for side in sides:
                    side.tick(lambda at: _fence(at, mark))
                if weigh:
                    pp.insert(0, weights(get_scores(j2, KB // G - 1 - g, half[t2 % 2]), m))
                    lsum = _fold8(lsum, pp[0], jnp.add)
            if weigh:
                p = jnp.concatenate(pp, axis=0).astype(bf16)
            acc = (nothing if j == 0 else acc) + o
            if j == NS - 1:
                oc[i, hd, 0:DH, :] = acc
                oc[i, hd, DH:DH + 8, :] = ldone
        return m, mn, lsum, p

    def softmax_attention(first):
        def block(i, c):
            def got_q(g, r, y):
                qT[g, i, r] = y.T.astype(bf16)

            def got_v(g, r, y):
                vT[g, i * 4 + r] = y.T.astype(bf16)

            def got_k(r, c, g, y):
                for t in range(2):
                    at = i * 4 + r, slice(g * RG, (g + 1) * RG)
                    kk[(4 * c + 2 * t,) + at] = y[:, _tile(t)].astype(bf16)
                    kk[(4 * c + 2 * t + 1,) + at] = pltpu.roll(y[:, _tile(t)], 2 * DH, 1).astype(bf16)

            sides = operand_sides(W_BQ, W_BQ, norm_jobs(xr, jnp.minimum(i + 1, NRB - 1)), room_b, 0.5)
            if first:
                n = KQ // NRB
                r0 = pl.multiple_of(i * n, 16)
                sides.append(_Side(rhs_jobs(INNER, wfa.at[4, :, :, pl.ds(r0, n)], 3, r0, n), 14 * T7, 5 * T7, room_b))
            project(W_BQ, sides, _by_tile(got_q, lambda c, y: y * QSCALE))
            project(W_BV, sides, _by_tile(got_v))
            project(W_BK, sides, got_k)
            drain()

        def park(state):
            for c in range(4):
                pc[c] = state[3][:, _tile(c)]
            return state[:3]

        def resume(carry):
            return carry + (jnp.concatenate([_packed(pc, c) for c in range(4)], axis=1),)

        def heads(i, carry):
            state = resume(carry)
            return park(attend(2 * i + 2, 0, attend(2 * i + 1, 1, state)))

        lax.fori_loop(0, NRB, block, None)
        _run(key_jobs(head(0, 0)))
        widen_q(head(0, 0), 1, 1)
        mn = [None] * 4
        for n in range(NS + 1):
            i, j = divmod(n, NS)
            s = qk(head(0, 0), i, j)
            for g in range(KB // G):
                put_scores(s[g * G:(g + 1) * G], j, g, i)
            if n == NS:
                m, mn = row_max(mn), [None] * 4
            mn = fold_max(mn, s)
        p = weights(jnp.concatenate([get_scores(0, g, 0) for g in range(KB // G)], axis=0), m)
        state = m, mn, _fold8(None, p, jnp.add), p.astype(bf16)
        state = resume(lax.fori_loop(0, H // 2 - 1, heads, park(attend(0, 0, state))))
        attend(H - 1, 1, state, [_Side(head_jobs(softmax_den, zero), 48 * 8),
                                 _Side(lhs_jobs(W_BO, ORDER[:AHEAD]), 14 * 8, 49 * 8)])
        out_project(W_BO, softmax_den, xr, not first)

    clear_summaries()
    for first in (True, False):
        linear_attention(first)
        softmax_attention(first)
    for c in [out_copy(i) for i in range(NRB - 1)] + sum(tail_cp, []):
        c.wait()


@jax.jit
def pallas_interleave_layers__linear_attn_block__mha_block__prompt_kernel(
    A_x: jax.Array,
    A_wqkv: jax.Array,
    A_wo: jax.Array,
    B_x: jax.Array,
    B_wqkv: jax.Array,
    B_wo: jax.Array,
):
    del B_x
    assert A_x.shape == (1, S, D)
    out = pl.pallas_call(
        _kernel,
        name="fused",
        out_shape=jax.ShapeDtypeStruct((S, D), bf16),
        in_specs=[pl.BlockSpec(memory_space=pl.ANY)] * 5,
        out_specs=pl.BlockSpec(memory_space=pl.ANY),
        scratch_shapes=[
            pltpu.VMEM((5, NPROD, 2, KQ, 128), bf16),
            pltpu.VMEM((3, NPROD, 2, KQ, 128), bf16),
            pltpu.VMEM((NPROD, 2, MQ, 128), bf16),
            pltpu.VMEM((D, D), bf16),
            pltpu.VMEM((4 * D + 16, D), bf16),
            pltpu.VMEM((S + 16, D), bf16),
            pltpu.VMEM((S + 8, D), f32),
            pltpu.VMEM((RB + 8, D), f32),
            pltpu.VMEM((NRB, H + 1, DH + 8, RB), f32),
            pltpu.VMEM((2, NG, 4, 128, 128), bf16),
            pltpu.VMEM((NG, 128, 128), f32),
            pltpu.VMEM((8, D), f32),
            pltpu.VMEM((D, 128), f32),
            pltpu.VMEM((NG, NRB, 4, 128, 128), bf16),
            pltpu.VMEM((H // 2, NS, KB, 128), bf16),
            pltpu.VMEM((NG, NS, 128, KB), bf16),
            pltpu.VMEM((4, KB, 128), bf16),
            pltpu.VMEM((1, 2 * (NV // 2 + 1), G, 128), f32),
            pltpu.VMEM((1, NV, DH, G, 128), f32),
            pltpu.VMEM((1, NV, DH, G, 128), f32),
            pltpu.SemaphoreType.DMA((NRB + 7 + 4 * len(WK_SPLIT),)),
        ] + [pltpu.VMEM((2, JB + 1, KB // 2, RB), f32)] * (2 * NS // JB),
        compiler_params=pltpu.CompilerParams(vmem_limit_bytes=126 * 2**20),
    )(A_x.reshape(S, D), A_wqkv, A_wo, B_wqkv, B_wo)
    return out.reshape(1, S, D)
```

```python
import math

import jax
import jax.numpy as jnp
from jax import lax
from jax.experimental import pallas as pl
from jax.experimental.pallas import tpu as pltpu

f32, bf16, u32 = jnp.float32, jnp.bfloat16, jnp.uint32

S, D, H, DH = 2048, 1024, 32, 32
NG = D // 128
QSCALE = math.log2(math.e) * DH ** -0.5

RB = 512
NRB = S // RB
MQ, KQ = RB // 4, D // 4
NPROD = 49
TPP = 4
RG = MQ // TPP
T7 = 7 * TPP
LAG = 4
AHEAD = 2
LN_ROWS, LN_GAP = 8, 4

KB = 128
NS = S // KB
G = 16
NV = 3
JB = 4

W_AQ, W_AK, W_AV, W_AO, W_BQ, W_BK, W_BV, W_BO = range(8)


def _tree(xs, op):
    while len(xs) > 1:
        xs = [op(xs[i], xs[i + 1]) if i + 1 < len(xs) else xs[i] for i in range(0, len(xs), 2)]
    return xs[0]


def _fold8(acc, x, op):
    x = _tree([x[i:i + 8] for i in range(0, x.shape[0], 8)], op)
    return x if acc is None else op(acc, x)


def _dot(a, b):
    return jnp.dot(a, b, preferred_element_type=f32)


def _packed(ref, *idx):
    return pltpu.bitcast(ref.bitcast(u32)[idx], bf16)


def _tile(c):
    return slice(128 * c, 128 * c + 128)


def _phi(t):
    return jnp.where(t > 0, t + 1.0, jnp.exp(t)) + 1e-6


_LHS = [[(1, 0, 0), (1, 1, 1)], [(1, 1, 0), (1, 1, 1)], [(1, 0, 0)], [(1, 1, 1)],
        [(1, 0, 0), (1, 0, 1)], [(1, 1, 0), (-1, 0, 0)], [(1, 0, 1), (-1, 1, 1)]]
_RHS = [[(1, 0, 0), (1, 1, 1)], [(1, 0, 0)], [(1, 0, 1), (-1, 1, 1)], [(1, 1, 0), (-1, 0, 0)],
        [(1, 1, 1)], [(1, 0, 0), (1, 0, 1)], [(1, 1, 0), (1, 1, 1)]]
ORDER = (0, 1, 3, 4, 2, 6, 5)


def _flip(table, rows, cols):
    return [[(s * (-1 if rows and r else 1) * (-1 if cols and c else 1), r, c) for s, r, c in t] for t in table]


ROWS = (_flip(_LHS, True, False), _RHS, -1)
INNER = (_flip(_LHS, False, True), _flip(_RHS, True, False), 1)
KIND = [ROWS] * 3 + [INNER] * 5


def _signed_sum(terms):
    s0, x = terms[0]
    for s, v in terms[1:]:
        x = x + v if s == s0 else x - v
    return s0, x


def _forms(table, i, block):
    q = {(r, c): _signed_sum([(s, block(2 * ro + r, 2 * co + c)) for s, ro, co in table[i]])[1]
         for r in range(2) for c in range(2)}
    return [_signed_sum([(s, q[r, c]) for s, r, c in t])[1] for t in table]


def _strassen(kind, prod, sink, lev=2, base=0):
    if lev == 0:
        return prod(base, lambda g, m: sink(0, 0, g, m))
    h = 2 ** (lev - 1)
    lhs, rhs, low = kind
    sg = [a[0][0] * b[0][0] for a, b in zip(lhs, rhs)]
    m1, m2, m5, c11, c22 = {}, {}, {}, {}, {}

    def total(*terms):
        s, x = _signed_sum(sorted(terms, key=lambda t: -t[0]))
        assert s > 0
        return x

    def got4(r, c, g, m):
        sink(h + r, c, g, total((low * sg[1], m2[r, c, g]), (low * sg[3], m)))
        c11[r, c, g] = total((sg[0], m1[r, c, g]), (sg[3], m))

    def got3(r, c, g, m):
        sink(r, h + c, g, total((sg[4], m5[r, c, g]), (sg[2], m)))
        c22[r, c, g] = total((sg[2], m), (sg[0], m1[r, c, g]), (-sg[1], m2[r, c, g]))

    got = [lambda r, c, g, m: m1.update({(r, c, g): m}),
           lambda r, c, g, m: m2.update({(r, c, g): m}),
           got3,
           got4,
           lambda r, c, g, m: m5.update({(r, c, g): m}),
           lambda r, c, g, m: sink(h + r, h + c, g, total((low * sg[5], m), (low, c22[r, c, g]))),
           lambda r, c, g, m: sink(r, c, g, total((sg[6], m), (1, c11[r, c, g]), (-sg[4], m5[r, c, g])))]
    for i in ORDER:
        _strassen(kind, prod, got[i], lev - 1, base + i * 7 ** (lev - 1))


def _by_tile(sink, pre=lambda c, y: y):
    parts = {}

    def part(r, c, g, y):
        parts.setdefault((r, c), []).append(pre(c, y))
        if g == TPP - 1:
            y = jnp.concatenate(parts.pop((r, c)), axis=0)
            for t in range(2):
                sink(2 * c + t, r, y[:, _tile(t)])
    return part


class _Side:
    def __init__(self, jobs, span, start=0, room=None):
        room = room[start:start + span] if room else [1] * span
        self.jobs, self.n, self.done, self.due, used = list(jobs), -start, 0, [], 0
        for r in room:
            used += r
            self.due.append(len(self.jobs) * used // sum(room))

    def tick(self, fence):
        while 0 <= self.n < len(self.due) and self.done < self.due[self.n]:
            self.jobs[self.done](fence)
            self.done += 1
        self.n += 1


def _room(*busy):
    final = (2, 4, 5, 6)
    return [10] * LAG + [b if o in final and i in final else 10
                         for b in busy for o in range(7) for i in range(7) for _ in range(TPP)]


def _staggered(gens, phases):
    def job(n):
        for k in reversed(range(phases)):
            if 0 <= n - k < len(gens):
                next(gens[n - k], None)
    return [lambda n=n: job(n) for n in range(len(gens) + phases - 1)]


def _fence(at, y):
    ref, rows = at[0], at[-1]
    ref[at[1:] + (slice(0, 128),)] = y[0:rows.stop - rows.start, 0:128].astype(ref.dtype)


def _fenced(at, jobs):
    def run(fence, job):
        fence(at)
        job()
    return [lambda fence, job=job: run(fence, job) for job in jobs]


def _run(jobs):
    for job in jobs:
        job(lambda at: None)


def _kernel(x_hbm, wa_hbm, woa_hbm, wb_hbm, wob_hbm, out_hbm,
            wfa, wfb, af, woa, raw, xio, xr, st, oc, pv, kv, zs, zb, qT, kk, vT, pc, kf, kb0, kb1, sem, *sb):
    wf = [(wfa, 0), (wfa, 1), (wfa, 2), (wfa, 3), (wfb, 0), (wfb, 1), (wfb, 2), (wfa, 4)]
    room_a, room_b, room_o = _room(0, 0, 1), _room(0, 0, 3), _room(1)

    def blk(i):
        return pl.ds(pl.multiple_of(i * RB, RB), RB)

    def x_copy(i):
        return pltpu.make_async_copy(x_hbm.at[blk(i)], xio.at[blk(i)], sem.at[i])

    def out_copy(i):
        return pltpu.make_async_copy(xio.at[blk(i)], out_hbm.at[blk(i)], sem.at[i])

    def wa_copy(w, c, n, s):
        return pltpu.make_async_copy(wa_hbm.at[:, pl.ds(w * D + c, n)], raw.at[pl.ds((1 + w) * D, D), pl.ds(c, n)],
                                     sem.at[NRB + 5 + s])

    x0_cp = [pltpu.make_async_copy(x_hbm.at[pl.ds(r, RB // 2)], xio.at[pl.ds(r, RB // 2)], sem.at[s])
             for r, s in ((0, 0), (RB // 2, NRB + 10))]
    wk_cp = [wa_copy(W_AK, 0, KQ, 0), wa_copy(W_AK, KQ, KQ, 1), wa_copy(W_AK, 2 * KQ, 2 * KQ, 2)]
    wq_cp, wv_cp = wa_copy(W_AQ, 0, D, 3), wa_copy(W_AV, 0, D, 4)
    wb_cp = [pltpu.make_async_copy(a, raw.at[pl.ds(t * D, D)], sem.at[NRB + t])
             for t, a in enumerate([wb_hbm.at[:, pl.ds(c * D, D)] for c in range(3)] + [wob_hbm])]
    wo_cp = pltpu.make_async_copy(woa_hbm, woa, sem.at[NRB + 4])
    corner = lambda ref, r, c: ref.at[pl.ds(S - RB + r * RB // 2, RB // 2), pl.ds(c * D // 2, D // 2)]
    tail_cp = [[pltpu.make_async_copy(corner(xio, r, c), corner(out_hbm, r, c), sem.at[NRB + 2 * r + c])
                for c in range(2)] for r in range(2)]

    for c in x0_cp + wk_cp + [wq_cp]:
        c.start()
    zero = lax.fori_loop(0, 2, lambda j, c: c + j // 8, 0)

    pending = []

    def issued(y, done, sides):
        for g in range(TPP):
            fence = lambda at: None
            if len(pending) >= LAG:
                fn, g0, y0 = pending.pop(0)
                fn(g0, y0)
                fence = lambda at: _fence(at, y0)
            for side in sides:
                side.tick(fence)
            pending.append((done, g, y[g * RG:(g + 1) * RG]))

    def project(w, sides, sink):
        def prod(p, done):
            issued(_dot(jnp.concatenate([_packed(af, p, c) for c in range(2)], axis=1),
                        jnp.concatenate([_packed(*wf[w], p, c) for c in range(2)], axis=1)), done, sides)
        _strassen(KIND[w], prod, sink)

    def drain():
        while pending:
            fn, g, y = pending.pop(0)
            fn(g, y)

    def form_jobs(table, dst, src, pitch, groups, rows):
        def job(r, c, i):
            tile = lambda a, b: src[a * pitch + r:a * pitch + r + 16, _tile(2 * b + c)].astype(f32)
            for j, f in enumerate(_forms(table, i, tile)):
                dst[7 * i + j, c, r:r + 16, :] = f.astype(bf16)
        todo = [(r, c, i) for i in groups for r in range(0, rows, 16) for c in range(2)]
        return [lambda t=t: job(*t) for t in (sorted(todo) if rows == 16 else todo)]

    def lhs_jobs(w, groups):
        return _fenced((st, slice(RB, RB + 8)), form_jobs(KIND[w][0], af, st.at[blk(zero)], MQ, groups, MQ))

    def rhs_jobs(kind, dst, slot, r0=0, rows=KQ):
        src = raw.at[pl.ds(pl.multiple_of(slot * D + r0, 16), D - KQ + rows)]
        return _fenced((raw, slice(4 * D, 4 * D + 16)), form_jobs(kind[1], dst, src, KQ, ORDER, rows))

    def operand_sides(w, w_next, fill, room, share):
        span = len(room) - LAG
        per = int(min(T7, span * (1.0 - share) / 7))
        a, b = (7 - AHEAD) * per, span - AHEAD * per
        return [_Side(lhs_jobs(w, ORDER[AHEAD:]), a, 0, room), _Side(fill, b - a - 4, a, room),
                _Side(lhs_jobs(w_next, ORDER[:AHEAD]), span - b - 2, b, room)]

    def norm_jobs(ref, i):
        src = ref.at[blk(i)]

        def rows(r):
            mu = jnp.mean(src[r, :].astype(f32), axis=-1, keepdims=True)
            for _ in range(LN_GAP):
                yield
            xc = src[r, :].astype(f32) - mu
            rstd = lax.rsqrt(jnp.mean(xc * xc, axis=-1, keepdims=True) + 1e-5)
            for _ in range(LN_GAP):
                yield
            st[r, :] = (src[r, :].astype(f32) - mu) * rstd
        return _fenced((ref, slice(S, ref.shape[0])),
                       _staggered([rows(slice(r, r + LN_ROWS)) for r in range(0, RB, LN_ROWS)], 2 * LN_GAP + 1))

    def head_jobs(denominator, i):
        def job(g, c):
            o = []
            for hd in range(4 * g, 4 * g + 4):
                x = oc[i, hd, 0:DH, _tile(c)]
                o.append(x * pltpu.reciprocal(denominator(x, i, hd, c), full_range=False))
            st[_tile(c), _tile(g)] = jnp.concatenate(o, axis=0).T
        return _fenced((oc, 0, H, slice(0, 8)), [lambda g=g, c=c: job(g, c) for g in range(NG) for c in range(4)])

    def linear_den(x, i, hd, c):
        return jnp.sum(_fold8(None, x * zb[DH * hd:DH * hd + DH, :], jnp.add), axis=0, keepdims=True) + 1e-6

    def softmax_den(x, i, hd, c):
        return jnp.sum(oc[i, hd, DH:DH + 8, _tile(c)], axis=0, keepdims=True)

    def out_project(w, den, x, final):
        def block(i, sides, last=False):
            src, dst = x.at[blk(i)], (xio if final else xr).at[blk(i)]

            def sink(r, c, g, y):
                at = slice(r * MQ + g * RG, r * MQ + (g + 1) * RG), slice(c * KQ, (c + 1) * KQ)
                dst[at] = (src[at].astype(f32) + y).astype(dst.dtype)
                if last and (r % 2, c % 2, g) == (1, 1, TPP - 1):
                    tail_cp[r // 2][c // 2].start()

            project(w, sides, sink)
            drain()
            if final and not last:
                out_copy(i).start()

        lax.fori_loop(0, NRB - 1, lambda i, c: block(i, operand_sides(w, w, head_jobs(den, i + 1), room_o, 0.4)), None)
        sides = operand_sides(w, (w + 1) % 8, norm_jobs(xr, zero), room_o, 0.55)
        if w == W_BO and not final:
            clear_summaries()
        block(zero + NRB - 1, sides[:1] if final else sides, final)

    def clear_summaries():
        kv[...] = jnp.zeros_like(kv)
        zs[...] = jnp.zeros_like(zs)

    def linear_block(i, mul):
        def phi_k(c, y):
            y = _phi(y)
            zs[:, c * KQ:(c + 1) * KQ] += _fold8(None, y, jnp.add)
            return y

        def got_k(g, r, y):
            pv[0, g, r] = y.T.astype(bf16)

        def got_q(g, r, y):
            y = _phi(y.T)
            for h in range(4):
                oc[i, 4 * g + h, 0:DH, _tile(r)] = y[DH * h:DH * h + DH]

        def got_v(r, c, g, y):
            for t in range(2):
                pv[1, 2 * c + t, r, g * RG:(g + 1) * RG, :] = y[:, _tile(t)].astype(bf16)

        mul(W_AK, _by_tile(got_k, phi_k))
        mul(W_AQ, _by_tile(got_q))
        mul(W_AV, got_v)
        for g in range(NG):
            if g == NG // 2:
                drain()
            kv[g] += _dot(jnp.concatenate([_packed(pv, 0, g, r) for r in range(4)], axis=1),
                          pltpu.bitcast(pv.bitcast(u32)[1, g].reshape(RB // 2, 128), bf16))

    def first_block():
        def arrive(at, done, new):
            def job(fence):
                for c in done:
                    c.wait()
                for c in new:
                    c.start()
            return _Side([job], 1, at - 1)

        def plain(sink):
            n = 16 * TPP
            room = [10] * LAG + ([10] * (3 * TPP) + [3] * TPP) * 16
            build = [_Side(lhs_jobs(W_AK, ORDER), 2 * n - 4, 0, room),
                     arrive(n, wk_cp[1:2], []), arrive(2 * n, wk_cp[2:], [wv_cp, x_copy(1)]),
                     _Side(rhs_jobs(ROWS, wfa.at[W_AK], zero + 1 + W_AK), 2 * n, 2 * n, room)]
            for c in range(4):
                for r in range(4):
                    part = {}
                    for k, t in ((0, 0), (0, 1), (4, 0), (4, 1)):
                        def done(g, y, r=r, c=c, k=k, t=t, part=part):
                            part[t, g] = part[t, g] + y if k else y
                            if k and t:
                                sink(r, c, g, jnp.concatenate([part[0, g], part[1, g]], axis=1))

                        k0 = (1 + W_AK) * D + 128 * k
                        issued(_dot(jnp.concatenate([_packed(kk, k + e, r) for e in range(4)], axis=1),
                                    raw[k0:k0 + 512, _tile(2 * c + t)]), done, build)
            drain()

        def prepare_q(j, c):
            r = pl.multiple_of(16 * j, 16)
            _run(rhs_jobs(ROWS, wfa.at[W_AQ, :, :, pl.ds(r, 16)], 1 + W_AQ, r, 16))

        def mul(w, sink):
            if w == W_AK:
                wk_cp[0].wait()
                plain(sink)
                wq_cp.wait()
                lax.fori_loop(0, KQ // 16, prepare_q, None)
                wv_cp.wait()
            else:
                project(w, sides, sink)

        for r in range(4):
            if r % 2 == 0:
                x0_cp[r // 2].wait()
            x = xio[r * MQ:(r + 1) * MQ, :].astype(f32)
            x = x - jnp.mean(x, axis=-1, keepdims=True)
            x = x * lax.rsqrt(jnp.mean(x * x, axis=-1, keepdims=True) + 1e-5)
            st[r * MQ:(r + 1) * MQ, :] = x
            for g in range(NG):
                kk[g, r] = x[:, _tile(g)].astype(bf16)
        t, room = 17 * TPP, room_a[7 * T7:]
        sides = [_Side(rhs_jobs(ROWS, wfa.at[W_AV], zero + 1 + W_AV), 73 * TPP, 0, room),
                 arrive(t, [x_copy(1)], [wb_cp[0], x_copy(2)]),
                 _Side(norm_jobs(xio, zero + 1), 12 * T7 - t - 4, t, room),
                 _Side(lhs_jobs(W_AQ, ORDER[:AHEAD]), 2 * T7, 12 * T7, room)]
        linear_block(zero, mul)

    def linear_attention(first):
        def block(i, c):
            fill = norm_jobs(xio if first else xr, jnp.minimum(i + 1, NRB - 1))
            sides = operand_sides(W_AQ, W_AQ, fill, room_a, 0.5)
            if first:
                for n in range(1, NRB):
                    @pl.when(i == n)
                    def _():
                        wb_cp[n].start()
                        if n + 1 < NRB:
                            (x_copy(3) if n == 1 else wo_cp).start()
                            x_copy(n + 1).wait()
                        wb_cp[n - 1].wait()

                sides.append(_Side(rhs_jobs(INNER, wfb.at[i - 1], i - 1), 21 * T7, 0, room_a))
            linear_block(i, lambda w, sink: project(w, sides, sink))

        if first:
            first_block()
        lax.fori_loop(1 if first else 0, NRB, block, None)
        if first:
            wo_cp.wait()
            wb_cp[3].wait()

        z = jnp.sum(zs[...], axis=0, keepdims=True)
        for g in range(NG):
            zb[_tile(g), :] = jnp.broadcast_to(z[:, _tile(g)], (128, 128)).T
        own = lax.broadcasted_iota(jnp.int32, (16, 128), 1) < DH
        sides = [_Side(head_jobs(linear_den, zero), 24), _Side(lhs_jobs(W_AO, ORDER[:AHEAD]), 8, 24)]
        for r in range(0, KQ, 16):
            rows = []
            for a in range(4):
                g, r0 = divmod(a * KQ + r, 128)
                shift = -(r0 // DH * DH) % 128
                y = kv[g, r0:r0 + 16, :]
                rows.append(jnp.where(own, pltpu.roll(y, shift, 1) if shift else y, 0.0).astype(bf16))
            for c in range(2):
                folded = []
                for a in range(4):
                    k = (a * KQ + r) // DH * DH
                    w = jnp.concatenate([woa[k:k + DH, _tile(2 * b + c)] for b in range(4)], axis=1)
                    folded.append(_dot(rows[a], jnp.concatenate([w, jnp.zeros((128 - DH, 512), bf16)], axis=0)))
                for i in range(7):
                    for j, f in enumerate(_forms(INNER[1], i, lambda a, b: folded[a][:, _tile(b)])):
                        wfa[W_AO, 7 * i + j, c, r:r + 16, :] = f.astype(bf16)
                for side in sides:
                    side.tick(lambda at: _fence(at, folded[0]))
        out_project(W_AO, linear_den, xio if first else xr, False)

    half, also_zero = [zero, 1 - zero], 2 * zero
    short = [NS * (t + 1) // NV - 1 for t in range(NV)]
    slots = [(j, g) for j in range(1, NS) for g in range(KB // G)][:-3]
    due = [(2 * NV * 4 * DH * k + len(slots)) // (2 * len(slots)) for k in range(len(slots) + 1)]
    terms = {slot: range(due[k], due[k + 1]) for k, slot in enumerate(slots)}
    wanted = {}
    for (j, g), us in terms.items():
        for u in us:
            wanted.setdefault((j // JB * 2 + g % 2, u // (NV * DH)), j)

    def scores(j, g, item, cols=slice(None)):
        j = (j - (g == KB // G - 1)) % NS
        return sb[j // JB * 2 + g % 2], (item, j % JB, slice(g // 2 * G, g // 2 * G + G), cols)

    def put_scores(s, *where):
        ref, idx = scores(*where)
        ref[idx] = s

    def get_scores(*where):
        ref, idx = scores(*where)
        return ref[idx]

    def head(hd, odd):
        rows = lambda n: pl.ds(pl.multiple_of((hd & 3) * n, n), n)
        return hd, odd, hd >> 1, hd >> 2, rows(DH), rows(DH // 2)

    def qk(h, i, j, rows=KB):
        q = jnp.concatenate([qT.bitcast(u32)[h[3], i, c, h[5]] for c in range(4)], axis=1)
        q = jnp.concatenate([q if a == h[1] else jnp.zeros_like(q) for a in range(4)], axis=0)
        return _dot(_packed(kk, h[2], j, slice(0, rows // 2)), pltpu.bitcast(q, bf16))

    def widen_q(h, i, j):
        for (a, c), j0 in wanted.items():
            if j0 == j:
                sb[a][zero, JB, 0:DH, _tile(c)] = qT[h[3], i, c, h[4], :].astype(f32)

    def key_jobs(h):
        def job(t, d):
            lane = h[1] * DH + d
            (kb0, kb1)[h[1]][0, t, d] = jnp.broadcast_to(kf[zero, t][:, lane:lane + 1], (G, 128))

        for t, j in enumerate(short):
            kf[0, t] = kk[h[2], j, KB - G:KB, :].astype(f32)
        return _fenced((kf, 0, NV, slice(0, 8)), [lambda t=t, d=d: job(t, d) for d in range(DH) for t in range(NV)])

    def row_max(m):
        return jnp.broadcast_to(jnp.max(jnp.concatenate(m, axis=1), axis=0, keepdims=True), (8, RB))

    def fold_max(m, s):
        s = _fold8(None, s, jnp.maximum)
        return [s[:, _tile(c)] if x is None else jnp.maximum(x, s[:, _tile(c)]) for c, x in enumerate(m)]

    def weights(s, m):
        return jnp.exp2(s.reshape(s.shape[0] // 8, 8, RB) - m[None]).reshape(s.shape)

    def attend(hd, odd, state, sides=None):
        last = sides is not None
        this, nxt = head(hd, odd), head(hd + 1, 1 - odd)
        sides = sides if last else [_Side(key_jobs(nxt), 28 * 8, 2 * 8)]
        m, mn, lsum, p = state
        partial, nothing = [], jnp.full((DH, RB), zero.astype(f32))
        for n in range(NRB * NS):
            i, j = divmod(n, NS)
            t1, j1 = divmod(n + NS + 1, NS)
            t2, j2 = divmod(n + 1, NS)
            h1 = this if t1 < NRB else nxt
            score, weigh, cut = not last or t1 < NRB, not last or t2 < NRB, j1 in short
            if score:
                widen_q(h1, t1 % NRB, j1 + 1)
                s = qk(h1, t1 % NRB, j1, KB - G if cut else KB)
            o = _dot(_packed(vT, this[3], j, this[5]), p)
            if j1 == 0:
                ldone, lsum = lsum, None
                if weigh:
                    m, mn = row_max(mn), [None] * 4
            pp = []
            for g in range(KB // G):
                mark = o
                if score:
                    near = sb[j1 // JB * 2 + g % 2]
                    for u in terms.get((j1, g), ()):
                        c, t, d = u // (NV * DH), u // DH % NV, u % DH
                        y = (kb0, kb1)[h1[1]][zero, t, d] * near[also_zero, JB, d:d + 1, _tile(c)]
                        sv = y if d == 0 else sv + y
                        if d == DH - 1:
                            mn[c] = _fold8(mn[c], sv, jnp.maximum)
                            put_scores(sv, short[t], KB // G - 1, half[t1 % 2], _tile(c))
                    if (j1, g) in terms:
                        partial.append(sv)
                        if len(partial) == 2:
                            near[half[t1 % 2], JB, DH:DH + G, 0:128] = partial.pop(0)
                    if not (cut and g == KB // G - 1):
                        mark = s[g * G:(g + 1) * G]
                        put_scores(mark, j1, g, half[t1 % 2])
                        mn = fold_max(mn, mark)
                for side in sides:
                    side.tick(lambda at: _fence(at, mark))
                if weigh:
                    pp.insert(0, weights(get_scores(j2, KB // G - 1 - g, half[t2 % 2]), m))
                    lsum = _fold8(lsum, pp[0], jnp.add)
            if weigh:
                p = jnp.concatenate(pp, axis=0).astype(bf16)
            acc = (nothing if j == 0 else acc) + o
            if j == NS - 1:
                oc[i, hd, 0:DH, :] = acc
                oc[i, hd, DH:DH + 8, :] = ldone
        return m, mn, lsum, p

    def softmax_attention(first):
        def block(i, c):
            def got_q(g, r, y):
                qT[g, i, r] = y.T.astype(bf16)

            def got_v(g, r, y):
                vT[g, i * 4 + r] = y.T.astype(bf16)

            def got_k(r, c, g, y):
                for t in range(2):
                    at = i * 4 + r, slice(g * RG, (g + 1) * RG)
                    kk[(4 * c + 2 * t,) + at] = y[:, _tile(t)].astype(bf16)
                    kk[(4 * c + 2 * t + 1,) + at] = pltpu.roll(y[:, _tile(t)], 2 * DH, 1).astype(bf16)

            sides = operand_sides(W_BQ, W_BQ, norm_jobs(xr, jnp.minimum(i + 1, NRB - 1)), room_b, 0.5)
            if first:
                n = KQ // NRB
                r0 = pl.multiple_of(i * n, 16)
                sides.append(_Side(rhs_jobs(INNER, wfa.at[4, :, :, pl.ds(r0, n)], 3, r0, n), 14 * T7, 5 * T7, room_b))
            project(W_BQ, sides, _by_tile(got_q, lambda c, y: y * QSCALE))
            project(W_BV, sides, _by_tile(got_v))
            project(W_BK, sides, got_k)
            drain()

        def park(state):
            for c in range(4):
                pc[c] = state[3][:, _tile(c)]
            return state[:3]

        def resume(carry):
            return carry + (jnp.concatenate([_packed(pc, c) for c in range(4)], axis=1),)

        def heads(i, carry):
            state = resume(carry)
            return park(attend(2 * i + 2, 0, attend(2 * i + 1, 1, state)))

        lax.fori_loop(0, NRB, block, None)
        _run(key_jobs(head(0, 0)))
        widen_q(head(0, 0), 1, 1)
        mn = [None] * 4
        for n in range(NS + 1):
            i, j = divmod(n, NS)
            s = qk(head(0, 0), i, j)
            for g in range(KB // G):
                put_scores(s[g * G:(g + 1) * G], j, g, i)
            if n == NS:
                m, mn = row_max(mn), [None] * 4
            mn = fold_max(mn, s)
        p = weights(jnp.concatenate([get_scores(0, g, 0) for g in range(KB // G)], axis=0), m)
        state = m, mn, _fold8(None, p, jnp.add), p.astype(bf16)
        state = resume(lax.fori_loop(0, H // 2 - 1, heads, park(attend(0, 0, state))))
        attend(H - 1, 1, state, [_Side(head_jobs(softmax_den, zero), 48 * 8),
                                 _Side(lhs_jobs(W_BO, ORDER[:AHEAD]), 14 * 8, 49 * 8)])
        out_project(W_BO, softmax_den, xr, not first)

    clear_summaries()
    for first in (True, False):
        linear_attention(first)
        softmax_attention(first)
    for c in [out_copy(i) for i in range(NRB - 1)] + sum(tail_cp, []):
        c.wait()


@jax.jit
def pallas_interleave_layers__linear_attn_block__mha_block__prompt_kernel(
    A_x: jax.Array,
    A_wqkv: jax.Array,
    A_wo: jax.Array,
    B_x: jax.Array,
    B_wqkv: jax.Array,
    B_wo: jax.Array,
):
    del B_x
    assert A_x.shape == (1, S, D)
    out = pl.pallas_call(
        _kernel,
        name="fused",
        out_shape=jax.ShapeDtypeStruct((S, D), bf16),
        in_specs=[pl.BlockSpec(memory_space=pl.ANY)] * 5,
        out_specs=pl.BlockSpec(memory_space=pl.ANY),
        scratch_shapes=[
            pltpu.VMEM((5, NPROD, 2, KQ, 128), bf16),
            pltpu.VMEM((3, NPROD, 2, KQ, 128), bf16),
            pltpu.VMEM((NPROD, 2, MQ, 128), bf16),
            pltpu.VMEM((D, D), bf16),
            pltpu.VMEM((4 * D + 16, D), bf16),
            pltpu.VMEM((S + 16, D), bf16),
            pltpu.VMEM((S + 8, D), f32),
            pltpu.VMEM((RB + 8, D), f32),
            pltpu.VMEM((NRB, H + 1, DH + 8, RB), f32),
            pltpu.VMEM((2, NG, 4, 128, 128), bf16),
            pltpu.VMEM((NG, 128, 128), f32),
            pltpu.VMEM((8, D), f32),
            pltpu.VMEM((D, 128), f32),
            pltpu.VMEM((NG, NRB, 4, 128, 128), bf16),
            pltpu.VMEM((H // 2, NS, KB, 128), bf16),
            pltpu.VMEM((NG, NS, 128, KB), bf16),
            pltpu.VMEM((4, KB, 128), bf16),
            pltpu.VMEM((1, 2 * (NV // 2 + 1), G, 128), f32),
            pltpu.VMEM((1, NV, DH, G, 128), f32),
            pltpu.VMEM((1, NV, DH, G, 128), f32),
            pltpu.SemaphoreType.DMA((NRB + 11,)),
        ] + [pltpu.VMEM((2, JB + 1, KB // 2, RB), f32)] * (2 * NS // JB),
        compiler_params=pltpu.CompilerParams(vmem_limit_bytes=126 * 2**20),
    )(A_x.reshape(S, D), A_wqkv, A_wo, B_wqkv, B_wo)
    return out.reshape(1, S, D)
```
